```python
import jax
import jax.numpy as jnp

def _softmax(x, axis=-1):
    return jax.nn.softmax(x, axis=axis)

def _gelu(x):
    return jax.nn.gelu(x, approximate=True)

def _silu(x):
    return jax.nn.silu(x)

def _sigmoid(x):
    return jax.nn.sigmoid(x)

def _layernorm(x, axis=-1, eps=1e-05):
    m = jnp.mean(x, axis=axis, keepdims=True)
    v = jnp.var(x, axis=axis, keepdims=True)
    return (x - m) / jnp.sqrt(v + eps)

def _scatter_add(tgt, idx, src, axis=0):
    return tgt.at[idx].add(src)

def _segment_sum(src, seg, n):
    return jax.ops.segment_sum(src, seg, n)

class _Rng:

    def __init__(self, key):
        self._k = key

    def _next(self):
        self._k, sub = jax.random.split(self._k)
        return sub

    def normal(self, shape):
        return jax.random.normal(self._next(), shape, dtype=jnp.bfloat16)

    def randint(self, lo, hi, shape):
        return jax.random.randint(self._next(), shape, lo, hi, dtype=jnp.int32)

    def uniform(self, shape, lo=0.0, hi=1.0):
        return jax.random.uniform(self._next(), shape, jnp.bfloat16, lo, hi)

    def permutation(self, n):
        return jax.random.permutation(self._next(), n)
kernel_name = 'interleave_layers__memory_aug_recurrent_mem_tr__sliding_local_dilated__prompt'

def setup_inputs():
    _rng = _Rng(jax.random.key(int.from_bytes(__import__("os").urandom(4), "little")))
    _w = lambda a: (lambda t: t.astype(jnp.bfloat16) if jnp.issubdtype(t.dtype, jnp.floating) else t)(jnp.asarray(a))

    def _A_setup():
        B, S, Dm = (1, 2048, 640)
        H, Dh = (32, 192)
        M, seg = (8, 32)
        seg = min(seg, S)
        S = S // seg * seg
        return {'x': _w((lambda *s: _rng.normal(s) * 0.05)(B, S, Dm)), 'mem0': _w((lambda *s: _rng.normal(s) * 0.05)(B, M, Dm)), 'Wq': _w((lambda *s: _rng.normal(s) * 0.05)(Dm, H, Dh) * Dm ** (-0.5)), 'Wk': _w((lambda *s: _rng.normal(s) * 0.05)(Dm, H, Dh) * Dm ** (-0.5)), 'Wv': _w((lambda *s: _rng.normal(s) * 0.05)(Dm, H, Dh) * Dm ** (-0.5)), 'Wo': _w((lambda *s: _rng.normal(s) * 0.05)(H, Dh, Dm) * (H * Dh) ** (-0.5)), 'seg_len': seg}
    _A_in = _A_setup()

    def _B_setup():
        B, S, D = (1, 2048, 640)
        return {'x': _w((lambda *s: _rng.normal(s) * 0.05)(B, S, D)), 'wqkv': _w((lambda *s: _rng.normal(s) * 0.05)(D, 3 * D)), 'wo': _w((lambda *s: _rng.normal(s) * 0.05)(D, D))}
    _B_in = _B_setup()
    return {'A_x': _A_in['x'], 'A_mem0': _A_in['mem0'], 'A_Wq': _A_in['Wq'], 'A_Wk': _A_in['Wk'], 'A_Wv': _A_in['Wv'], 'A_Wo': _A_in['Wo'], 'A_seg_len': _A_in['seg_len'], 'B_x': _B_in['x'], 'B_wqkv': _B_in['wqkv'], 'B_wo': _B_in['wo']}

def reference(A_x, A_mem0, A_Wq, A_Wk, A_Wv, A_Wo, A_seg_len, B_x, B_wqkv, B_wo):

    def _A_ref(x, mem0, Wq, Wk, Wv, Wo, seg_len):
        B, S, Dm = x.shape
        H, Dh = (Wq.shape[1], Wq.shape[2])
        M = mem0.shape[1]
        scale = Dh ** (-0.5)
        n_seg = S // seg_len
        L = M + seg_len
        idx = jnp.arange(L)
        mask = (idx[:, None] < M) | (idx[:, None] >= idx[None, :])
        mem = mem0
        outs = []
        for s in range(n_seg):
            xs = x[:, s * seg_len:(s + 1) * seg_len, :].copy()
            h = jnp.concatenate([mem, xs], axis=1)
            q = jnp.einsum('btd,dhe->bhte', h, Wq)
            k = jnp.einsum('btd,dhe->bhte', h, Wk)
            v = jnp.einsum('btd,dhe->bhte', h, Wv)
            scores = jnp.einsum('bhqe,bhke->bhqk', q, k) * scale
            scores = jnp.where(mask[None, None], scores, -1000000000.0)
            p = _softmax(scores, axis=-1)
            o = jnp.einsum('bhqk,bhke->bhqe', p, v)
            o = jnp.einsum('bhte,hed->btd', o, Wo)
            mem = o[:, :M, :].copy()
            outs.append(o[:, M:, :])
        return jnp.concatenate(outs, axis=1)

    def _B_ref(x, wqkv, wo):
        B, S, D = x.shape
        H = 32
        Dh = D // H
        W, dil = (8, 2)
        qkv = (lambda x, *d: x.transpose(*d))((x @ wqkv).reshape(B, S, 3, H, Dh), 2, 0, 3, 1, 4)
        q, k, v = (qkv[0], qkv[1], qkv[2])
        scale = Dh ** (-0.5)
        pos = jnp.arange(S)
        off = jnp.arange(W) * dil
        idx = pos[:, None] - off[None, :]
        mask = idx >= 0
        idx_c = jnp.where(mask, idx, 0).reshape(-1)
        kg = k[:, :, idx_c, :].reshape(B, H, S, W, Dh)
        vg = v[:, :, idx_c, :].reshape(B, H, S, W, Dh)
        logits = jnp.einsum('bhsd,bhswd->bhsw', q, kg) * scale
        logits = jnp.where(mask[None, None, :, :], logits, -1000000000.0)
        attn = _softmax(logits, axis=-1)
        o = jnp.einsum('bhsw,bhswd->bhsd', attn, vg)
        return (lambda x, *d: x.transpose(*d))(o, 0, 2, 1, 3).reshape(B, S, D) @ wo
    x = A_x
    x = x + _A_ref(_layernorm(x, axis=-1), A_mem0, A_Wq, A_Wk, A_Wv, A_Wo, A_seg_len)
    x = x + _B_ref(_layernorm(x, axis=-1), B_wqkv, B_wo)
    x = x + _A_ref(_layernorm(x, axis=-1), A_mem0, A_Wq, A_Wk, A_Wv, A_Wo, A_seg_len)
    x = x + _B_ref(_layernorm(x, axis=-1), B_wqkv, B_wo)
    return x
```

```python
import functools

import jax
import jax.numpy as jnp
from jax import lax
import jax.experimental.pallas as pl
import jax.experimental.pallas.tpu as pltpu

F32 = jnp.float32
BF16 = jnp.bfloat16
U32 = jnp.uint32

S = 2048
D = 640
SEG = 32
M = 8
NSEG = S // SEG
L = SEG + M
H = 32
DH = 192
NP = H // 2
NT = H * DH // 128
KT = D // 128
BW = 8
BDIL = 2
BDH = D // H
HIST = 16
NEG = -1000000000.0
EPS = 1e-5
NCH = 8
AHEAD = 3
SCHEDULE = "K0 K1 PV-2 K2 KP Q0 Q1 Q2 B V0 V1 QK V2 VP B O0-3 S1-1 O1-3 O2-3 S2-1 O3-3 O4-3 S3-1 B"


def _bf(x):
    return pltpu.bitcast(x, BF16)


def _u32(x):
    return pltpu.bitcast(x, U32)


def _dot(a, b):
    return lax.dot_general(a, b, (((1,), (0,)), ((), ())), preferred_element_type=F32)


def _dot_t(a, b):
    return lax.dot_general(a, b, (((1,), (1,)), ((), ())), preferred_element_type=F32)


def _layernorm(x):
    m = jnp.sum(x, axis=-1, keepdims=True) * (1.0 / D)
    c = x - m
    v = jnp.sum(c * c, axis=-1, keepdims=True) * (1.0 / D)
    return c * lax.rsqrt(v + EPS)


def _recip(l):
    r = pl.reciprocal(l, approx=True)
    return r * (2.0 - l * r)


def _softmax_rows(s):
    m = jnp.max(s, axis=-1, keepdims=True)
    p = jnp.exp(s - m)
    l = jnp.sum(p, axis=-1, keepdims=True)
    return p * _recip(l)


def _kernel(x_hbm, mem0_hbm, wqt_hbm, wkt_hbm, wvt_hbm, wo_hbm, bqkv_hbm, bwo_hbm,
            out_ref,
            xs, mem_s, x_s, h_s, stq, stk, stv, wq, wk, wv, wo,
            bst_qkv, bst_o, bqkv, bwo, kprev, vprev,
            sem_small, sem_a, sem_o):
    CR = H * DH // NCH
    wob = wo.bitcast(BF16)

    def a_copies(c):
        rows = pl.ds(c * CR, CR)
        return [pltpu.make_async_copy(src.at[rows, :], dst.at[rows, :], sem_a.at[c, wi])
                for wi, (src, dst) in enumerate(((wqt_hbm, stq), (wkt_hbm, stk), (wvt_hbm, stv)))]

    def first_layernorm():
        def init_rows(i, _):
            r = pl.ds(pl.multiple_of(i * 128, 128), 128)
            xv = xs[r, :].astype(F32)
            x_s[r, :] = xv
            h_s[r, :] = _layernorm(xv)
            return 0
        lax.fori_loop(0, S // 128, init_rows, 0)

    ri = lax.broadcasted_iota(jnp.int32, (D, D), 0)
    ci = lax.broadcasted_iota(jnp.int32, (D, D), 1)

    def permute_qkv(part):
        perm = jnp.where(ri == (ci & 31) * BDH + (ci >> 5), 1.0, 0.0).astype(BF16)
        wp = _dot(bst_qkv[:, part * D:(part + 1) * D], perm).astype(BF16)
        for j in range(KT):
            bqkv[part * KT + j] = _u32(wp[:, j * 128:(j + 1) * 128])

    def permute_wo():
        permt = jnp.where(ci == (ri & 31) * BDH + (ri >> 5), 1.0, 0.0).astype(BF16)
        wp = _dot(permt, bst_o[...]).astype(BF16)
        for j in range(KT):
            bwo[j] = _u32(wp[:, j * 128:(j + 1) * 128])

    def transpose_chunk(c):
        ei = lax.broadcasted_iota(jnp.int32, (128, 128), 0)
        ej = lax.broadcasted_iota(jnp.int32, (128, 128), 1)
        eye = jnp.where(ei == ej, 1.0, 0.0).astype(BF16)

        def tr_tile(j, _):
            r = pl.ds(pl.multiple_of(j * 128, 128), 128)
            for st, w in ((stq, wq), (stk, wk), (stv, wv)):
                for i in range(KT):
                    t = _dot_t(eye, st[r, i * 128:(i + 1) * 128]).astype(BF16)
                    w[j, i * 64:(i + 1) * 64, :] = _u32(t)
            return 0
        lax.fori_loop(c * (NT // NCH), (c + 1) * (NT // NCH), tr_tile, 0)

    items = [
        ([pltpu.make_async_copy(x_hbm, xs, sem_small.at[0]),
          pltpu.make_async_copy(mem0_hbm, mem_s, sem_small.at[1])], [first_layernorm]),
        ([pltpu.make_async_copy(bqkv_hbm, bst_qkv, sem_small.at[2]),
          pltpu.make_async_copy(bwo_hbm, bst_o, sem_small.at[3])], [functools.partial(permute_qkv, 0)]),
    ]
    extra = [functools.partial(permute_qkv, 1), functools.partial(permute_qkv, 2), permute_wo]
    for c in range(NCH):
        work = [functools.partial(transpose_chunk, c)]
        if c < len(extra):
            work.append(extra[c])
        items.append((a_copies(c), work))
    for j in range(KT):
        items.append(([pltpu.make_async_copy(wo_hbm.at[:, pl.ds(j * 128, 128)], wob.at[j], sem_o.at[j])], []))

    for copies, _ in items[:AHEAD]:
        for cp in copies:
            cp.start()

    kprev[...] = jnp.zeros(kprev.shape, F32)
    vprev[...] = jnp.zeros(vprev.shape, F32)
    x_s[pl.ds(S, SEG), :] = jnp.zeros((SEG, D), F32)
    h_s[pl.ds(S, SEG), :] = jnp.zeros((SEG, D), F32)

    for n, (copies, work) in enumerate(items):
        if n + AHEAD < len(items):
            for cp in items[n + AHEAD][0]:
                cp.start()
        for cp in copies:
            cp.wait()
        for fn in work:
            fn()

    mem0 = jnp.concatenate([mem_s[...].astype(F32)], axis=0)

    lane = lax.broadcasted_iota(jnp.int32, (L, 128), 1)
    lo_half = lane < 64
    arow = lax.broadcasted_iota(jnp.int32, (L, 2 * L), 0)
    acol = lax.broadcasted_iota(jnp.int32, (L, 2 * L), 1)
    akey = jnp.where(acol < L, acol, acol - L)
    allowed = (arow >= SEG) | (akey >= SEG) | (akey <= arow)
    mask_e = allowed & (acol < L)
    mask_o = allowed & (acol >= L)
    a_scale = DH ** -0.5
    b_scale = BDH ** -0.5

    brow = lax.broadcasted_iota(jnp.int32, (SEG, 128), 0)

    def b_stages(u):
        seg = jnp.where(u < 0, NSEG, u % NSEG)
        r = pl.ds(pl.multiple_of(seg * SEG, SEG), SEG)
        xrows = x_s[r, :]
        hn = _layernorm(xrows)
        yield
        k = []
        for j in range(KT):
            k.append(_dot(hn, _bf(bqkv[KT + j])))
            yield
        kp = kprev[...]
        kwin = [jnp.concatenate([kp[:, j * 128:(j + 1) * 128], k[j]], axis=0) for j in range(KT)]
        for j in range(KT):
            kprev[:, j * 128:(j + 1) * 128] = k[j][SEG - HIST:]
        q = []
        for j in range(KT):
            q.append(_dot(hn, _bf(bqkv[j])))
            yield
        pos = brow + seg * SEG
        logits = []
        for w in range(BW):
            off = HIST - BDIL * w
            t = q[0] * kwin[0][off:off + SEG]
            for j in range(1, KT):
                t = t + q[j] * kwin[j][off:off + SEG]
            t = t + pltpu.roll(t, 64, axis=1)
            t = t + pltpu.roll(t, 32, axis=1)
            logits.append(jnp.where(pos >= BDIL * w, t * b_scale, NEG))
            yield
        m = logits[0]
        for w in range(1, BW):
            m = jnp.maximum(m, logits[w])
        e = [jnp.exp(lg - m) for lg in logits]
        l = e[0]
        for w in range(1, BW):
            l = l + e[w]
        rl = _recip(l)
        a = [ew * rl for ew in e]
        yield
        vp = vprev[...]
        o = []
        for j in range(KT):
            vj = _dot(hn, _bf(bqkv[2 * KT + j]))
            yield
            vwin = jnp.concatenate([vp[:, j * 128:(j + 1) * 128], vj], axis=0)
            vprev[:, j * 128:(j + 1) * 128] = vj[SEG - HIST:]
            t = a[0] * vwin[HIST:HIST + SEG]
            for w in range(1, BW):
                off = HIST - BDIL * w
                t = t + a[w] * vwin[off:off + SEG]
            o.append(t)
            yield
        o = jnp.concatenate(o, axis=1)
        y = []
        for j in range(KT):
            y.append(_dot(o, _bf(bwo[j])))
            yield
        xn = xrows + jnp.concatenate(y, axis=1)
        x_s[r, :] = xn
        h_s[r, :] = _layernorm(xn)
        yield

    def advance(gen, n):
        for _ in range(n):
            next(gen, None)

    def a_layer(hrows, bgen):
        st = [dict() for _ in range(NP)]
        acc = [None] * KT

        def pack_kv(t):
            ac = jnp.concatenate([t[0], t[2]], axis=0).astype(BF16)
            bb = jnp.concatenate([jnp.where(lo_half, t[1], 0.0),
                                  jnp.where(lo_half, 0.0, t[1])], axis=0).astype(BF16)
            return ac, bb

        def run(op, p):
            d = st[p]
            if op[0] in "KQV" and op[1] in "012":
                w = {"K": wk, "Q": wq, "V": wv}[op[0]]
                d.setdefault(op[0], {})[int(op[1])] = _dot(hrows, _bf(w[3 * p + int(op[1])]))
            elif op == "KP":
                d["kp"] = pack_kv(d.pop("K"))
            elif op == "VP":
                d["vp"] = pack_kv(d.pop("V"))
            elif op == "QK":
                q = d.pop("Q")
                k_ac, k_b = d.pop("kp")
                d["sc"] = (_dot_t(jnp.concatenate([q[0], q[2]], axis=0), k_ac), _dot_t(q[1], k_b))
            elif op == "S1":
                s_ac, s_b = d.pop("sc")
                s_e = jnp.where(mask_e, (s_ac[:L] + s_b) * a_scale, NEG)
                s_o = jnp.where(mask_o, (s_ac[L:] + s_b) * a_scale, NEG)
                d["mx"] = [(s, jnp.max(s, axis=-1, keepdims=True)) for s in (s_e, s_o)]
            elif op == "S2":
                es = [jnp.exp(s - m) for s, m in d.pop("mx")]
                d["pr"] = [(e, jnp.sum(e, axis=-1, keepdims=True)) for e in es]
            elif op == "S3":
                d["p"] = [e * _recip(l) for e, l in d.pop("pr")]
            elif op == "PV":
                p_e, p_o = d.pop("p")
                v_ac, v_b = d.pop("vp")
                o_ac = _dot(jnp.concatenate([p_e, p_o], axis=0), v_ac)
                o_b = _dot(p_e + p_o, v_b)
                d["o"] = jnp.concatenate([o_ac[:L], o_b, o_ac[L:]], axis=1)
            elif op[0] == "O":
                j = int(op[1])
                part = _dot(d["o"], _bf(wo[j, 192 * p:192 * (p + 1), :]))
                acc[j] = part if acc[j] is None else acc[j] + part
            else:
                raise ValueError(op)

        maxlag = max(int(t.partition("-")[2] or 0) for t in SCHEDULE.split())
        for i in range(NP + maxlag):
            for tok in SCHEDULE.split():
                if tok == "B":
                    advance(bgen, 1)
                    continue
                op, _, lag = tok.partition("-")
                p = i - int(lag or 0)
                if 0 <= p < NP:
                    run(op, p)
        return jnp.concatenate(acc, axis=1)

    def step(u, mem):
        seg = u % NSEG
        mem = jnp.where(seg == 0, mem0, mem)
        r = pl.ds(pl.multiple_of(seg * SEG, SEG), SEG)
        hrows = jnp.concatenate([h_s[r, :], mem], axis=0)
        bgen = b_stages(u - 1)
        y = a_layer(hrows, bgen)
        advance(bgen, 1000)
        x_s[r, :] = x_s[r, :] + y[:SEG]
        return y[SEG:]

    lax.fori_loop(0, 2 * NSEG, step, mem0)
    advance(b_stages(2 * NSEG - 1), 1000)

    def write_rows(i, _):
        r = pl.ds(pl.multiple_of(i * 128, 128), 128)
        out_ref[r, :] = x_s[r, :].astype(BF16)
        return 0
    lax.fori_loop(0, S // 128, write_rows, 0)


@functools.partial(jax.jit, static_argnames=("A_seg_len",))
def pallas_interleave_layers__memory_aug_recurrent_mem_tr__sliding_local_dilated__prompt_kernel(
    A_x, A_mem0, A_Wq, A_Wk, A_Wv, A_Wo, A_seg_len, B_x, B_wqkv, B_wo,
):
    del B_x
    assert int(A_seg_len) == SEG
    assert A_x.shape == (1, S, D) and A_mem0.shape == (1, M, D)
    assert A_Wq.shape == (D, H, DH) and A_Wo.shape == (H, DH, D)

    def wt(w):
        return jnp.transpose(w, (1, 2, 0)).reshape(H * DH, D)

    any_spec = pl.BlockSpec(memory_space=pl.ANY)
    out = pl.pallas_call(
        _kernel,
        out_shape=jax.ShapeDtypeStruct((S, D), BF16),
        in_specs=[any_spec] * 8,
        out_specs=pl.BlockSpec(memory_space=pltpu.VMEM),
        scratch_shapes=[
            pltpu.VMEM((S, D), BF16),
            pltpu.VMEM((M, D), BF16),
            pltpu.VMEM((S + SEG, D), F32),
            pltpu.VMEM((S + SEG, D), F32),
            pltpu.VMEM((H * DH, D), BF16),
            pltpu.VMEM((H * DH, D), BF16),
            pltpu.VMEM((H * DH, D), BF16),
            pltpu.VMEM((NT, D // 2, 128), U32),
            pltpu.VMEM((NT, D // 2, 128), U32),
            pltpu.VMEM((NT, D // 2, 128), U32),
            pltpu.VMEM((KT, H * DH // 2, 128), U32),
            pltpu.VMEM((D, 3 * D), BF16),
            pltpu.VMEM((D, D), BF16),
            pltpu.VMEM((3 * KT, D // 2, 128), U32),
            pltpu.VMEM((KT, D // 2, 128), U32),
            pltpu.VMEM((HIST, D), F32),
            pltpu.VMEM((HIST, D), F32),
            pltpu.SemaphoreType.DMA((4,)),
            pltpu.SemaphoreType.DMA((NCH, 3)),
            pltpu.SemaphoreType.DMA((KT,)),
        ],
        compiler_params=pltpu.CompilerParams(vmem_limit_bytes=120 * 1024 * 1024),
        name="interleaved_rmt_dilated",
    )(A_x.reshape(S, D), A_mem0.reshape(M, D), wt(A_Wq), wt(A_Wk), wt(A_Wv),
      A_Wo.reshape(H * DH, D), B_wqkv, B_wo)
    return out.reshape(1, S, D)
```

```python
import functools

import jax
import jax.numpy as jnp
from jax import lax
import jax.experimental.pallas as pl
import jax.experimental.pallas.tpu as pltpu

F32 = jnp.float32
BF16 = jnp.bfloat16
U32 = jnp.uint32

S = 2048
D = 640
SEG = 32
M = 8
NSEG = S // SEG
L = SEG + M
H = 32
DH = 192
NP = H // 2
NT = H * DH // 128
KT = D // 128
BW = 8
BDIL = 2
BDH = D // H
HIST = 16
NEG = -1000000000.0
EPS = 1e-5
UNROLL = 1
BCOUNT = (2, 1, 2, 1, 2, 1, 2, 1, 2, 1, 2, 1, 2, 0, 1, 0, 4, 4, 2)
NCH = 8
AHEAD = 2
SCHEDULE = "K0 K1 PV-2 K2 KP Q0 Q1 Q2 B V0 V1 QK V2 VP B O0-3 S1-1 O1-3 O2-3 S2-1 O3-3 O4-3 S3-1 B"


def _bf(x):
    return pltpu.bitcast(x, BF16)


def _u32(x):
    return pltpu.bitcast(x, U32)


def _dot(a, b):
    return lax.dot_general(a, b, (((1,), (0,)), ((), ())), preferred_element_type=F32)


def _dot_t(a, b):
    return lax.dot_general(a, b, (((1,), (1,)), ((), ())), preferred_element_type=F32)


def _layernorm(x):
    m = jnp.sum(x, axis=-1, keepdims=True) * (1.0 / D)
    c = x - m
    v = jnp.sum(c * c, axis=-1, keepdims=True) * (1.0 / D)
    return c * lax.rsqrt(v + EPS)


def _recip(l):
    r = pl.reciprocal(l, approx=True)
    return r * (2.0 - l * r)


def _softmax_rows(s):
    m = jnp.max(s, axis=-1, keepdims=True)
    p = jnp.exp(s - m)
    l = jnp.sum(p, axis=-1, keepdims=True)
    return p * _recip(l)


def _kernel(x_hbm, mem0_hbm, wqt_hbm, wkt_hbm, wvt_hbm, wo_hbm, bqkv_hbm, bwo_hbm,
            out_ref,
            xs, mem_s, x_s, h_s, stq, stk, stv, wq, wk, wv, wo,
            bst_qkv, bst_o, bqkv, bwo, kwin, vwin, qbuf,
            sem_small, sem_a, sem_o, sem_out):
    CR = H * DH // NCH
    wob = wo.bitcast(BF16)

    def a_copies(c):
        rows = pl.ds(c * CR, CR)
        return [pltpu.make_async_copy(src.at[rows, :], dst.at[rows, :], sem_a.at[c, wi])
                for wi, (src, dst) in enumerate(((wqt_hbm, stq), (wkt_hbm, stk), (wvt_hbm, stv)))]

    def first_layernorm():
        def init_rows(i, _):
            r = pl.ds(pl.multiple_of(i * 128, 128), 128)
            xv = xs[r, :].astype(F32)
            x_s[r, :] = xv
            h_s[r, :] = _layernorm(xv)
            return 0
        lax.fori_loop(0, S // 128, init_rows, 0)

    ri = lax.broadcasted_iota(jnp.int32, (D, D), 0)
    ci = lax.broadcasted_iota(jnp.int32, (D, D), 1)

    def permute_qkv(part):
        perm = jnp.where(ri == (ci & 31) * BDH + (ci >> 5), 1.0, 0.0).astype(BF16)
        wp = _dot(bst_qkv[:, part * D:(part + 1) * D], perm).astype(BF16)
        for j in range(KT):
            bqkv[part * KT + j] = _u32(wp[:, j * 128:(j + 1) * 128])

    def permute_wo():
        permt = jnp.where(ci == (ri & 31) * BDH + (ri >> 5), 1.0, 0.0).astype(BF16)
        wp = _dot(permt, bst_o[...]).astype(BF16)
        for j in range(KT):
            bwo[j] = _u32(wp[:, j * 128:(j + 1) * 128])

    def transpose_chunk(c):
        ei = lax.broadcasted_iota(jnp.int32, (128, 128), 0)
        ej = lax.broadcasted_iota(jnp.int32, (128, 128), 1)
        eye = jnp.where(ei == ej, 1.0, 0.0).astype(BF16)

        def tr_tile(j, _):
            r = pl.ds(pl.multiple_of(j * 128, 128), 128)
            for st, w in ((stq, wq), (stk, wk), (stv, wv)):
                for i in range(KT):
                    t = _dot_t(eye, st[r, i * 128:(i + 1) * 128]).astype(BF16)
                    w[j, i * 64:(i + 1) * 64, :] = _u32(t)
            return 0
        lax.fori_loop(c * (NT // NCH), (c + 1) * (NT // NCH), tr_tile, 0)

    def wo_copies(c):
        rows = pl.ds(c * CR, CR)
        return [pltpu.make_async_copy(wo_hbm.at[rows, pl.ds(j * 128, 128)], wob.at[j, rows, :],
                                      sem_o.at[c, j]) for j in range(KT)]

    items = [
        ([pltpu.make_async_copy(x_hbm, xs.at[pl.ds(0, S), :], sem_small.at[0]),
          pltpu.make_async_copy(mem0_hbm, mem_s, sem_small.at[1])], [first_layernorm]),
        ([pltpu.make_async_copy(bqkv_hbm, bst_qkv, sem_small.at[2]),
          pltpu.make_async_copy(bwo_hbm, bst_o, sem_small.at[3])], [functools.partial(permute_qkv, 0)]),
    ]
    extra = [functools.partial(permute_qkv, 1), functools.partial(permute_qkv, 2), permute_wo]
    for c in range(NCH):
        work = [functools.partial(transpose_chunk, c)]
        if c < len(extra):
            work.append(extra[c])
        items.append((a_copies(c) + wo_copies(c), work))

    def run_item(n):
        copies, work = items[n]
        if n + AHEAD < len(items):
            for cp in items[n + AHEAD][0]:
                cp.start()
        for cp in copies:
            cp.wait()
        for fn in work:
            fn()

    for copies, _ in items[:AHEAD]:
        for cp in copies:
            cp.start()

    kwin[...] = jnp.zeros(kwin.shape, F32)
    vwin[...] = jnp.zeros(vwin.shape, F32)
    qbuf[...] = jnp.zeros(qbuf.shape, F32)
    x_s[pl.ds(S, SEG), :] = jnp.zeros((SEG, D), F32)
    h_s[pl.ds(S, SEG), :] = jnp.zeros((SEG, D), F32)
    run_item(0)
    run_item(1)

    mem0 = jnp.concatenate([mem_s[...].astype(F32)], axis=0)

    lane = lax.broadcasted_iota(jnp.int32, (L, 128), 1)
    lo_half = lane < 64
    arow = lax.broadcasted_iota(jnp.int32, (L, 2 * L), 0)
    acol = lax.broadcasted_iota(jnp.int32, (L, 2 * L), 1)
    akey = jnp.where(acol < L, acol, acol - L)
    allowed = (arow >= SEG) | (akey >= SEG) | (akey <= arow)
    mask_e = allowed & (acol < L)
    mask_o = allowed & (acol >= L)
    a_scale = DH ** -0.5
    b_scale = BDH ** -0.5

    brow = lax.broadcasted_iota(jnp.int32, (SEG, 128), 0)

    def seg_rows(seg):
        if isinstance(seg, int):
            return pl.ds(seg * SEG, SEG)
        return pl.ds(pl.multiple_of(seg * SEG, SEG), SEG)

    def b_rows(u):
        if isinstance(u, int):
            seg = NSEG if u < 0 else u % NSEG
        else:
            seg = jnp.where(u < 0, NSEG, u % NSEG)
        return seg, seg_rows(seg)

    def b_first(u):
        _, r = b_rows(u)
        hn = _layernorm(x_s[r, :])
        kwin[0:HIST, :] = kwin[SEG:SEG + HIST, :]
        vwin[0:HIST, :] = vwin[SEG:SEG + HIST, :]
        yield
        for j in range(KT):
            kwin[HIST:, j * 128:(j + 1) * 128] = _dot(hn, _bf(bqkv[KT + j]))
            yield
        for j in range(KT):
            qbuf[:, j * 128:(j + 1) * 128] = _dot(hn, _bf(bqkv[j]))
            yield
        for j in range(KT):
            vwin[HIST:, j * 128:(j + 1) * 128] = _dot(hn, _bf(bqkv[2 * KT + j]))
            yield

    def b_second(u):
        seg, r = b_rows(u)
        pos = brow + seg * SEG
        logits = []
        for w in range(BW):
            off = HIST - BDIL * w
            t = None
            for j in range(KT):
                cols = slice(j * 128, (j + 1) * 128)
                pj = qbuf[:, cols] * kwin[off:off + SEG, cols]
                t = pj if t is None else t + pj
            t = t + pltpu.roll(t, 64, axis=1)
            t = t + pltpu.roll(t, 32, axis=1)
            logits.append(jnp.where(pos >= BDIL * w, t * b_scale, NEG))
            yield
        m = logits[0]
        for w in range(1, BW):
            m = jnp.maximum(m, logits[w])
        e = [jnp.exp(lg - m) for lg in logits]
        l = e[0]
        for w in range(1, BW):
            l = l + e[w]
        rl = _recip(l)
        a = [ew * rl for ew in e]
        yield
        o = []
        for j in range(KT):
            cols = slice(j * 128, (j + 1) * 128)
            t = None
            for w in range(BW):
                off = HIST - BDIL * w
                pw = a[w] * vwin[off:off + SEG, cols]
                t = pw if t is None else t + pw
            o.append(t)
            yield
        o = jnp.concatenate(o, axis=1)
        y = []
        for j in range(KT):
            y.append(_dot(o, _bf(bwo[j])))
            yield
        xn = x_s[r, :] + jnp.concatenate(y, axis=1)
        x_s[r, :] = xn
        xs[r, :] = xn.astype(BF16)
        h_s[r, :] = _layernorm(xn)
        yield

    def chain(*gens):
        for g in gens:
            yield from g

    def advance(gen, n):
        for _ in range(n):
            next(gen, None)

    def a_layer(hrows, bgen, weights_ready=None):
        st = [dict() for _ in range(NP)]
        acc = [None] * KT

        def pack_kv(t):
            ac = jnp.concatenate([t[0], t[2]], axis=0).astype(BF16)
            bb = jnp.concatenate([jnp.where(lo_half, t[1], 0.0),
                                  jnp.where(lo_half, 0.0, t[1])], axis=0).astype(BF16)
            return ac, bb

        def run(op, p):
            d = st[p]
            if op[0] in "KQV" and op[1] in "012":
                w = {"K": wk, "Q": wq, "V": wv}[op[0]]
                d.setdefault(op[0], {})[int(op[1])] = _dot(hrows, _bf(w[3 * p + int(op[1])]))
            elif op == "KP":
                d["kp"] = pack_kv(d.pop("K"))
            elif op == "VP":
                d["vp"] = pack_kv(d.pop("V"))
            elif op == "QK":
                q = d.pop("Q")
                k_ac, k_b = d.pop("kp")
                d["sc"] = (_dot_t(jnp.concatenate([q[0], q[2]], axis=0), k_ac), _dot_t(q[1], k_b))
            elif op == "S1":
                s_ac, s_b = d.pop("sc")
                s_e = jnp.where(mask_e, (s_ac[:L] + s_b) * a_scale, NEG)
                s_o = jnp.where(mask_o, (s_ac[L:] + s_b) * a_scale, NEG)
                d["mx"] = [(s, jnp.max(s, axis=-1, keepdims=True)) for s in (s_e, s_o)]
            elif op == "S2":
                es = [jnp.exp(s - m) for s, m in d.pop("mx")]
                d["pr"] = [(e, jnp.sum(e, axis=-1, keepdims=True)) for e in es]
            elif op == "S3":
                d["p"] = [e * _recip(l) for e, l in d.pop("pr")]
            elif op == "PV":
                p_e, p_o = d.pop("p")
                v_ac, v_b = d.pop("vp")
                o_ac = _dot(jnp.concatenate([p_e, p_o], axis=0), v_ac)
                o_b = _dot(p_e + p_o, v_b)
                d["o"] = jnp.concatenate([o_ac[:L], o_b, o_ac[L:]], axis=1)
            elif op[0] == "O":
                j = int(op[1])
                part = _dot(d["o"], _bf(wo[j, 192 * p:192 * (p + 1), :]))
                acc[j] = part if acc[j] is None else acc[j] + part
            else:
                raise ValueError(op)

        toks = SCHEDULE.split()
        maxlag = max(int(t.partition("-")[2] or 0) for t in toks)
        nb = toks.count("B")
        for i in range(NP + maxlag):
            bi = 0
            if weights_ready is not None and i < NP and i % (NP // NCH) == 0:
                weights_ready(i // (NP // NCH))
            for tok in toks:
                if tok == "B":
                    n = BCOUNT[i]
                    advance(bgen, (n * (bi + 1)) // nb - (n * bi) // nb)
                    bi += 1
                    continue
                op, _, lag = tok.partition("-")
                p = i - int(lag or 0)
                if 0 <= p < NP:
                    run(op, p)
        return jnp.concatenate(acc, axis=1)

    def out_copy(seg):
        r = seg_rows(seg)
        return pltpu.make_async_copy(xs.at[r, :], out_ref.at[r, :], sem_out.at[0])

    def step(u, mem, first=False):
        seg = u % NSEG
        if isinstance(u, int):
            mem = mem0 if seg == 0 else mem
        else:
            mem = jnp.where(seg == 0, mem0, mem)
        r = seg_rows(seg)
        hrows = jnp.concatenate([h_s[r, :], mem], axis=0)
        if first:
            y = a_layer(hrows, iter(()), lambda c: run_item(2 + c))
        else:
            bgen = chain(b_second(u - 2), b_first(u - 1))
            y = a_layer(hrows, bgen)
            advance(bgen, 1000)
        x_s[r, :] = x_s[r, :] + y[:SEG]
        if not first:
            @pl.when(u - 2 >= NSEG)
            def _():
                out_copy(u - 2 - NSEG).start()
        return y[SEG:]

    def steps(i, mem):
        for t in range(UNROLL):
            mem = step(1 + i * UNROLL + t, mem)
        return mem

    mem = step(0, mem0, first=True)
    nloop = (2 * NSEG - 1) // UNROLL
    mem = lax.fori_loop(0, nloop, steps, mem)
    for u in range(1 + nloop * UNROLL, 2 * NSEG):
        mem = step(u, mem)
    advance(chain(b_second(2 * NSEG - 2), b_first(2 * NSEG - 1), b_second(2 * NSEG - 1)), 1000)
    out_copy(NSEG - 2).start()
    out_copy(NSEG - 1).start()

    def wait_out(i, _):
        out_copy(i).wait()
        return 0
    lax.fori_loop(0, NSEG, wait_out, 0)


@functools.partial(jax.jit, static_argnames=("A_seg_len",))
def pallas_interleave_layers__memory_aug_recurrent_mem_tr__sliding_local_dilated__prompt_kernel(
    A_x, A_mem0, A_Wq, A_Wk, A_Wv, A_Wo, A_seg_len, B_x, B_wqkv, B_wo,
):
    del B_x
    assert int(A_seg_len) == SEG
    assert A_x.shape == (1, S, D) and A_mem0.shape == (1, M, D)
    assert A_Wq.shape == (D, H, DH) and A_Wo.shape == (H, DH, D)

    def wt(w):
        return jnp.transpose(w, (1, 2, 0)).reshape(H * DH, D)

    any_spec = pl.BlockSpec(memory_space=pl.ANY)
    out = pl.pallas_call(
        _kernel,
        out_shape=jax.ShapeDtypeStruct((S, D), BF16),
        in_specs=[any_spec] * 8,
        out_specs=any_spec,
        scratch_shapes=[
            pltpu.VMEM((S + SEG, D), BF16),
            pltpu.VMEM((M, D), BF16),
            pltpu.VMEM((S + SEG, D), F32),
            pltpu.VMEM((S + SEG, D), F32),
            pltpu.VMEM((H * DH, D), BF16),
            pltpu.VMEM((H * DH, D), BF16),
            pltpu.VMEM((H * DH, D), BF16),
            pltpu.VMEM((NT, D // 2, 128), U32),
            pltpu.VMEM((NT, D // 2, 128), U32),
            pltpu.VMEM((NT, D // 2, 128), U32),
            pltpu.VMEM((KT, H * DH // 2, 128), U32),
            pltpu.VMEM((D, 3 * D), BF16),
            pltpu.VMEM((D, D), BF16),
            pltpu.VMEM((3 * KT, D // 2, 128), U32),
            pltpu.VMEM((KT, D // 2, 128), U32),
            pltpu.VMEM((HIST + SEG, D), F32),
            pltpu.VMEM((HIST + SEG, D), F32),
            pltpu.VMEM((SEG, D), F32),
            pltpu.SemaphoreType.DMA((4,)),
            pltpu.SemaphoreType.DMA((NCH, 3)),
            pltpu.SemaphoreType.DMA((NCH, KT)),
            pltpu.SemaphoreType.DMA((1,)),
        ],
        compiler_params=pltpu.CompilerParams(vmem_limit_bytes=120 * 1024 * 1024),
        name="interleaved_rmt_dilated",
    )(A_x.reshape(S, D), A_mem0.reshape(M, D), wt(A_Wq), wt(A_Wk), wt(A_Wv),
      A_Wo.reshape(H * DH, D), B_wqkv, B_wo)
    return out.reshape(1, S, D)
```

```python
import functools

import jax
import jax.numpy as jnp
from jax import lax
import jax.experimental.pallas as pl
import jax.experimental.pallas.tpu as pltpu

F32 = jnp.float32
BF16 = jnp.bfloat16
U32 = jnp.uint32

S = 2048
D = 640
SEG = 32
M = 8
NSEG = S // SEG
L = SEG + M
H = 32
DH = 192
NQ = H // 4
QR = 4 * DH
KT = D // 128
BW = 8
BDIL = 2
BDH = D // H
HIST = 16
NEG = -1000000000.0
EPS = 1e-5
NSLOT = 3
AHEAD = 2
LAG = 2
BCOUNT = (16, 4, 4, 4, 4, 4, 4, 4, 5)
SCHEDULE = "K0 S3a-1 S3b-1 K1 S3c-1 B S3d-1 K2 PVa-1 PVb-1 KPa KPb PVc-1 PVd-1 KPc KPd B Q1 OC-1 Q2 B Q0 V0 QKa QKb QKc QKd V1 S1a S1b S1c S1d V2 OA-1 S2a VPa VPb B OB-1 S2d S2b VPc VPd OR-1 S2c"


def _bf(x):
    return pltpu.bitcast(x, BF16)


def _u32(x):
    return pltpu.bitcast(x, U32)


def _dot(a, b):
    return lax.dot_general(a, b, (((1,), (0,)), ((), ())), preferred_element_type=F32)


def _dot_t(a, b):
    return lax.dot_general(a, b, (((1,), (1,)), ((), ())), preferred_element_type=F32)


def _layernorm(x):
    m = jnp.sum(x, axis=-1, keepdims=True) * (1.0 / D)
    c = x - m
    v = jnp.sum(c * c, axis=-1, keepdims=True) * (1.0 / D)
    return c * lax.rsqrt(v + EPS)


def _recip(l):
    r = pl.reciprocal(l, approx=True)
    return r * (2.0 - l * r)


def _add(a, b):
    return b if a is None else a if b is None else a + b


def _sub(a, b):
    return a if b is None else (-b if a is None else a - b)


def _lhs_combos(a11, a12, a21, a22):
    return [_add(a11, a22), _add(a21, a22), a11, a22, _add(a11, a12), _sub(a21, a11), _sub(a12, a22)]


def _rhs_combos(b11, b12, b21, b22):
    return [b11 + b22, b11, b12 - b22, b21 - b11, b22, b11 + b12, b21 + b22]


def _needed(live1, live2):
    return sorted(({0, 2, 3, 4, 6} if live1 else set()) | ({0, 1, 2, 3, 5} if live2 else set()))


def _recombine(m, live1=True, live2=True):
    top = (_add(_sub(_add(m[0], m[3]), m[4]), m[6]), _add(m[2], m[4])) if live1 else (None, None)
    bot = (_add(m[1], m[3]), _add(_add(_sub(m[0], m[1]), m[2]), m[5])) if live2 else (None, None)
    return top + bot


def _kernel(x_hbm, mem0_hbm, wqt_hbm, wkt_hbm, wvt_hbm, wo_hbm, bqkv_hbm, bwo_hbm,
            out_ref,
            xs, mem_s, x_s, h_s, stage, ws, wso, wsr, lhs,
            bst_qkv, bst_o, bqkv, bwo, kwin, vwin,
            sem_small, sem_a, sem_out):
    def a_copies(c):
        rows = pl.ds(c * QR, QR)
        return [pltpu.make_async_copy(src.at[rows, :], stage.at[c % NSLOT, w], sem_a.at[c, w])
                for w, src in enumerate((wqt_hbm, wkt_hbm, wvt_hbm, wo_hbm))]

    def first_layernorm():
        def init_rows(i, _):
            r = pl.ds(pl.multiple_of(i * 128, 128), 128)
            xv = xs[r, :].astype(F32)
            x_s[r, :] = xv
            h_s[r, :] = _layernorm(xv)
            return 0
        lax.fori_loop(0, S // 128, init_rows, 0)

    ri = lax.broadcasted_iota(jnp.int32, (D, D), 0)
    ci = lax.broadcasted_iota(jnp.int32, (D, D), 1)

    def permute_qkv(part):
        perm = jnp.where(ri == (ci & 31) * BDH + (ci >> 5), 1.0, 0.0).astype(BF16)
        wp = _dot(bst_qkv[:, part * D:(part + 1) * D], perm).astype(BF16)
        for j in range(KT):
            bqkv[part * KT + j] = _u32(wp[:, j * 128:(j + 1) * 128])

    def permute_wo():
        permt = jnp.where(ci == (ri & 31) * BDH + (ri >> 5), 1.0, 0.0).astype(BF16)
        wp = _dot(permt, bst_o[...]).astype(BF16)
        for j in range(KT):
            bwo[j] = _u32(wp[:, j * 128:(j + 1) * 128])

    def build_chunk(c):
        slot = c % NSLOT
        ei = lax.broadcasted_iota(jnp.int32, (128, 128), 0)
        ej = lax.broadcasted_iota(jnp.int32, (128, 128), 1)
        eye = jnp.where(ei == ej, 1.0, 0.0).astype(BF16)

        def qkv_block(n, _):
            w = n // 3
            tt = n % 3
            idx = (w * NQ + c) * 3 + tt

            def tr(half, i):
                r = pl.ds(pl.multiple_of((3 * half + tt) * 128, 128), 128)
                return _dot_t(eye, stage[slot, w, r, i * 128:(i + 1) * 128])

            for ii in range(2):
                combos = _rhs_combos(tr(0, ii), tr(1, ii), tr(0, 2 + ii), tr(1, 2 + ii))
                for i, cmb in enumerate(combos):
                    ws[idx, i * 128 + ii * 64:i * 128 + (ii + 1) * 64, :] = _u32(cmb.astype(BF16))
            ws[idx, 896:960, :] = _u32(tr(0, 4).astype(BF16))
            ws[idx, 960:1024, :] = _u32(tr(1, 4).astype(BF16))
            return 0
        lax.fori_loop(0, 9, qkv_block, 0)

        def o_block(n, _):
            npair = n // 3
            r = n % 3
            c1 = pl.ds(pl.multiple_of(npair * 256, 256), 128)
            c2 = pl.ds(pl.multiple_of(npair * 256 + 128, 128), 128)
            r1 = pl.ds(pl.multiple_of(r * 128, 128), 128)
            r2 = pl.ds(pl.multiple_of(384 + r * 128, 128), 128)
            combos = _rhs_combos(stage[slot, 3, r1, c1].astype(F32), stage[slot, 3, r1, c2].astype(F32),
                                 stage[slot, 3, r2, c1].astype(F32), stage[slot, 3, r2, c2].astype(F32))
            for i, cmb in enumerate(combos):
                wso[c * 2 + npair, pl.ds(pl.multiple_of(i * 192 + r * 64, 64), 64), :] = _u32(cmb.astype(BF16))
            return 0
        lax.fori_loop(0, 6, o_block, 0)
        wsr[c] = _u32(stage[slot, 3, :, 512:640])

    items = [
        ([pltpu.make_async_copy(x_hbm, xs.at[pl.ds(0, S), :], sem_small.at[0]),
          pltpu.make_async_copy(mem0_hbm, mem_s, sem_small.at[1])], [first_layernorm]),
        ([pltpu.make_async_copy(bqkv_hbm, bst_qkv, sem_small.at[2]),
          pltpu.make_async_copy(bwo_hbm, bst_o, sem_small.at[3])], [functools.partial(permute_qkv, 0)]),
    ]
    extra = [functools.partial(permute_qkv, 1), functools.partial(permute_qkv, 2), permute_wo]
    for c in range(NQ):
        work = [functools.partial(build_chunk, c)]
        if c < len(extra):
            work.append(extra[c])
        items.append((a_copies(c), work))

    def run_item(n):
        copies, work = items[n]
        if n + AHEAD < len(items):
            for cp in items[n + AHEAD][0]:
                cp.start()
        for cp in copies:
            cp.wait()
        for fn in work:
            fn()

    for copies, _ in items[:AHEAD]:
        for cp in copies:
            cp.start()

    kwin[...] = jnp.zeros(kwin.shape, F32)
    vwin[...] = jnp.zeros(vwin.shape, F32)
    x_s[pl.ds(S, SEG), :] = jnp.zeros((SEG, D), F32)
    h_s[pl.ds(S, SEG), :] = jnp.zeros((SEG, D), F32)
    run_item(0)
    run_item(1)

    mem0 = mem_s[...].astype(F32)

    lane = lax.broadcasted_iota(jnp.int32, (L, 128), 1)
    lo_half = lane < 64
    arow = lax.broadcasted_iota(jnp.int32, (L, 2 * L), 0)
    acol = lax.broadcasted_iota(jnp.int32, (L, 2 * L), 1)
    akey = jnp.where(acol < L, acol, acol - L)
    allowed = (arow >= SEG) | (akey >= SEG) | (akey <= arow)
    mask_e = allowed & (acol < L)
    mask_o = allowed & (acol >= L)
    a_scale = DH ** -0.5
    b_scale = BDH ** -0.5
    brow = lax.broadcasted_iota(jnp.int32, (SEG, 128), 0)

    def seg_rows(seg):
        if isinstance(seg, int):
            return pl.ds(seg * SEG, SEG)
        return pl.ds(pl.multiple_of(seg * SEG, SEG), SEG)

    def b_stages(s1, s2):
        live = [n for n, sg in enumerate((s1, s2)) if sg is not None]
        if not live:
            return
        segs = {n: (s1, s2)[n] for n in live}
        rows = {n: seg_rows(segs[n]) for n in live}
        off_of = {n: i * SEG for i, n in enumerate(live)}
        hn = jnp.concatenate([_layernorm(x_s[rows[n], :]) for n in live], axis=0)
        for n in live:
            kwin[n, 0:HIST, :] = kwin[n, SEG:SEG + HIST, :]
            vwin[n, 0:HIST, :] = vwin[n, SEG:SEG + HIST, :]
        yield
        q = []
        for j in range(KT):
            cols = slice(j * 128, (j + 1) * 128)
            k = _dot(hn, _bf(bqkv[KT + j]))
            for n in live:
                kwin[n, HIST:, cols] = k[off_of[n]:off_of[n] + SEG]
            yield
        for j in range(KT):
            q.append(_dot(hn, _bf(bqkv[j])))
            yield
        for j in range(KT):
            cols = slice(j * 128, (j + 1) * 128)
            v = _dot(hn, _bf(bqkv[2 * KT + j]))
            for n in live:
                vwin[n, HIST:, cols] = v[off_of[n]:off_of[n] + SEG]
            yield
        o = {n: [None] * KT for n in live}
        for n in live:
            pos = brow + segs[n] * SEG
            logits = []
            for w in range(BW):
                off = HIST - BDIL * w
                t = None
                for j in range(KT):
                    cols = slice(j * 128, (j + 1) * 128)
                    pj = q[j][off_of[n]:off_of[n] + SEG] * kwin[n, off:off + SEG, cols]
                    t = pj if t is None else t + pj
                t = t + pltpu.roll(t, 64, axis=1)
                t = t + pltpu.roll(t, 32, axis=1)
                logits.append(jnp.where(pos >= BDIL * w, t * b_scale, NEG))
                yield
            m = logits[0]
            for w in range(1, BW):
                m = jnp.maximum(m, logits[w])
            e = [jnp.exp(lg - m) for lg in logits]
            l = e[0]
            for w in range(1, BW):
                l = l + e[w]
            rl = _recip(l)
            a = [ew * rl for ew in e]
            yield
            for j in range(KT):
                cols = slice(j * 128, (j + 1) * 128)
                t = None
                for w in range(BW):
                    off = HIST - BDIL * w
                    pw = a[w] * vwin[n, off:off + SEG, cols]
                    t = pw if t is None else t + pw
                o[n][j] = t
                yield
        o = jnp.concatenate([jnp.concatenate(o[n], axis=1) for n in live], axis=0)
        y = []
        for j in range(KT):
            y.append(_dot(o, _bf(bwo[j])))
            yield
        y = jnp.concatenate(y, axis=1)
        for n in live:
            xn = x_s[rows[n], :] + y[off_of[n]:off_of[n] + SEG]
            x_s[rows[n], :] = xn
            if n == 0:
                h_s[rows[n], :] = _layernorm(xn)
            else:
                xs[rows[n], :] = xn.astype(BF16)
        yield

    def advance(gen, n):
        for _ in range(n):
            next(gen, None)

    def a_layers(h1, h2, bgen, weights_ready=None):
        live1, live2 = h1 is not None, h2 is not None
        need = _needed(live1, live2)
        live_inst = ([0, 1] if live1 else []) + ([2, 3] if live2 else [])
        inst = [dict() for _ in range(4 * NQ)]
        acc_m = [[None] * 7, [None] * 7]
        acc_r = [None]
        blk = lambda h, j: None if h is None else h[:, 256 * j:256 * (j + 1)]
        have = {}
        for i, cmb in enumerate(_lhs_combos(blk(h1, 0), blk(h1, 1), blk(h2, 0), blk(h2, 1))):
            if i in need and cmb is not None:
                lhs[i] = cmb
                have[i] = True
        rem = jnp.concatenate([h[:, 512:] for h in (h1, h2) if h is not None], axis=0)

        def split_rows(r):
            if live1 and live2:
                return r[:L], r[L:]
            return (r, None) if live1 else (None, r)

        def pack_kv(t):
            ac = jnp.concatenate([t[0], t[2]], axis=0).astype(BF16)
            bb = jnp.concatenate([jnp.where(lo_half, t[1], 0.0),
                                  jnp.where(lo_half, 0.0, t[1])], axis=0).astype(BF16)
            return ac, bb

        def run(op, qd):
            if op[0] in "KQV" and op[1] in "012":
                tt = int(op[1])
                idx = ("QKV".index(op[0]) * NQ + qd) * 3 + tt
                mi = [_dot(lhs[i], _bf(ws[idx, 128 * i:128 * (i + 1), :])) if i in have else None
                      for i in range(7)]
                r1 = split_rows(_dot(rem, _bf(ws[idx, 896:960, :])))
                r2 = split_rows(_dot(rem, _bf(ws[idx, 960:1024, :])))
                c = _recombine(mi, live1, live2)
                for n, r in enumerate((r1[0], r2[0], r1[1], r2[1])):
                    if n in live_inst:
                        inst[qd * 4 + n].setdefault(op[0], {})[tt] = c[n] + r
                return
            if op == "OC":
                o = [inst[qd * 4 + n].pop("o") if n in live_inst else None for n in range(4)]
                inst[qd * 4]["oc"] = [cmb if i in need else None for i, cmb in enumerate(_lhs_combos(*o))]
                inst[qd * 4]["orem"] = jnp.concatenate(
                    [jnp.concatenate([o[2 * n], o[2 * n + 1]], axis=1) for n in range(2)
                     if o[2 * n] is not None], axis=0)
                return
            if op in ("OA", "OB"):
                npair = "AB".index(op[1])
                for i, cmb in enumerate(inst[qd * 4]["oc"]):
                    if cmb is not None:
                        part = _dot(cmb, _bf(wso[qd * 2 + npair, 192 * i:192 * (i + 1), :]))
                        acc_m[npair][i] = _add(acc_m[npair][i], part)
                return
            if op == "OR":
                part = _dot(inst[qd * 4].pop("orem"), _bf(wsr[qd]))
                acc_r[0] = _add(acc_r[0], part)
                return
            if "abcd".index(op[2]) not in live_inst:
                return
            d = inst[qd * 4 + "abcd".index(op[2])]
            op = op[:2]
            if op == "KP":
                d["kp"] = pack_kv(d.pop("K"))
            elif op == "VP":
                d["vp"] = pack_kv(d.pop("V"))
            elif op == "QK":
                q = d.pop("Q")
                k_ac, k_b = d.pop("kp")
                d["sc"] = (_dot_t(jnp.concatenate([q[0], q[2]], axis=0), k_ac), _dot_t(q[1], k_b))
            elif op == "S1":
                s_ac, s_b = d.pop("sc")
                s_e = jnp.where(mask_e, (s_ac[:L] + s_b) * a_scale, NEG)
                s_o = jnp.where(mask_o, (s_ac[L:] + s_b) * a_scale, NEG)
                d["mx"] = [(s, jnp.max(s, axis=-1, keepdims=True)) for s in (s_e, s_o)]
            elif op == "S2":
                es = [jnp.exp(s - m) for s, m in d.pop("mx")]
                d["pr"] = [(e, jnp.sum(e, axis=-1, keepdims=True)) for e in es]
            elif op == "S3":
                d["p"] = [e * _recip(l) for e, l in d.pop("pr")]
            elif op == "PV":
                p_e, p_o = d.pop("p")
                v_ac, v_b = d.pop("vp")
                o_ac = _dot(jnp.concatenate([p_e, p_o], axis=0), v_ac)
                o_b = _dot(p_e + p_o, v_b)
                d["o"] = jnp.concatenate([o_ac[:L], o_b, o_ac[L:]], axis=1)
            else:
                raise ValueError(op)

        toks = SCHEDULE.split()
        maxlag = max(int(t.partition("-")[2] or 0) for t in toks)
        nb = toks.count("B")
        for i in range(NQ + maxlag):
            if weights_ready is not None and i < NQ:
                weights_ready(i)
            bi = 0
            for tok in toks:
                if tok == "B":
                    n = BCOUNT[i] if i < len(BCOUNT) else 0
                    advance(bgen, (n * (bi + 1)) // nb - (n * bi) // nb)
                    bi += 1
                    continue
                op, _, lag = tok.partition("-")
                qd = i - int(lag or 0)
                if 0 <= qd < NQ:
                    run(op, qd)
        blocks = [_recombine(acc_m[npair], live1, live2) for npair in range(2)]
        r4 = split_rows(acc_r[0])
        y1 = y2 = None
        if live1:
            y1 = jnp.concatenate([blocks[0][0], blocks[0][1], blocks[1][0], blocks[1][1], r4[0]], axis=1)
        if live2:
            y2 = jnp.concatenate([blocks[0][2], blocks[0][3], blocks[1][2], blocks[1][3], r4[1]], axis=1)
        return y1, y2

    def out_copy(seg):
        r = seg_rows(seg)
        return pltpu.make_async_copy(xs.at[r, :], out_ref.at[r, :], sem_out.at[0])

    def step(t, carry, first=False):
        mem1, mem2 = carry
        static = isinstance(t, int)
        valid = lambda sg: sg if (not static or 0 <= sg < NSEG) else None
        s1, s2, sb1, sb2 = valid(t), valid(t - LAG), valid(t - 1), valid(t - LAG - 1)
        if not static:
            sb2 = jnp.where(sb2 < 0, NSEG, sb2)
        h1 = None if s1 is None else jnp.concatenate([h_s[seg_rows(s1), :], mem1], axis=0)
        h2 = None if s2 is None else jnp.concatenate([h_s[seg_rows(s2), :], mem2], axis=0)
        bgen = b_stages(sb1, sb2)
        y1, y2 = a_layers(h1, h2, bgen, (lambda c: run_item(2 + c)) if first else None)
        advance(bgen, 1000)
        if s1 is not None:
            x_s[seg_rows(s1), :] = x_s[seg_rows(s1), :] + y1[:SEG]
            mem1 = y1[SEG:]
        if s2 is not None:
            x_s[seg_rows(s2), :] = x_s[seg_rows(s2), :] + y2[:SEG]
            mem2 = y2[SEG:]
        if static:
            if sb2 is not None:
                out_copy(sb2).start()
        else:
            @pl.when(t - LAG - 1 >= 0)
            def _():
                out_copy(t - LAG - 1).start()
        return mem1, mem2

    carry = step(0, (mem0, mem0), first=True)
    for t in range(1, LAG):
        carry = step(t, carry)
    carry = lax.fori_loop(LAG, NSEG, step, carry)
    for t in range(NSEG, NSEG + LAG):
        carry = step(t, carry)
    advance(b_stages(None, NSEG - 1), 1000)
    out_copy(NSEG - 1).start()

    def wait_out(i, _):
        out_copy(i).wait()
        return 0
    lax.fori_loop(0, NSEG, wait_out, 0)


@functools.partial(jax.jit, static_argnames=("A_seg_len",))
def pallas_interleave_layers__memory_aug_recurrent_mem_tr__sliding_local_dilated__prompt_kernel(
    A_x, A_mem0, A_Wq, A_Wk, A_Wv, A_Wo, A_seg_len, B_x, B_wqkv, B_wo,
):
    del B_x
    assert int(A_seg_len) == SEG
    assert A_x.shape == (1, S, D) and A_mem0.shape == (1, M, D)
    assert A_Wq.shape == (D, H, DH) and A_Wo.shape == (H, DH, D)

    def wt(w):
        return jnp.transpose(w, (1, 2, 0)).reshape(H * DH, D)

    any_spec = pl.BlockSpec(memory_space=pl.ANY)
    out = pl.pallas_call(
        _kernel,
        out_shape=jax.ShapeDtypeStruct((S, D), BF16),
        in_specs=[any_spec] * 8,
        out_specs=any_spec,
        scratch_shapes=[
            pltpu.VMEM((S + SEG, D), BF16),
            pltpu.VMEM((M, D), BF16),
            pltpu.VMEM((S + SEG, D), F32),
            pltpu.VMEM((S + SEG, D), F32),
            pltpu.VMEM((NSLOT, 4, QR, D), BF16),
            pltpu.VMEM((3 * NQ * 3, 1024, 128), U32),
            pltpu.VMEM((NQ * 2, 7 * 192, 128), U32),
            pltpu.VMEM((NQ, QR // 2, 128), U32),
            pltpu.VMEM((7, L, 256), F32),
            pltpu.VMEM((D, 3 * D), BF16),
            pltpu.VMEM((D, D), BF16),
            pltpu.VMEM((3 * KT, D // 2, 128), U32),
            pltpu.VMEM((KT, D // 2, 128), U32),
            pltpu.VMEM((2, HIST + SEG, D), F32),
            pltpu.VMEM((2, HIST + SEG, D), F32),
            pltpu.SemaphoreType.DMA((4,)),
            pltpu.SemaphoreType.DMA((NQ, 4)),
            pltpu.SemaphoreType.DMA((1,)),
        ],
        compiler_params=pltpu.CompilerParams(vmem_limit_bytes=120 * 1024 * 1024),
        name="interleaved_rmt_dilated",
    )(A_x.reshape(S, D), A_mem0.reshape(M, D), wt(A_Wq), wt(A_Wk), wt(A_Wv),
      A_Wo.reshape(H * DH, D), B_wqkv, B_wo)
    return out.reshape(1, S, D)
```

```python
import functools

import jax
import jax.numpy as jnp
from jax import lax
import jax.experimental.pallas as pl
import jax.experimental.pallas.tpu as pltpu

F32 = jnp.float32
BF16 = jnp.bfloat16
U32 = jnp.uint32

S = 2048
D = 640
SEG = 32
M = 8
NSEG = S // SEG
L = SEG + M
H = 32
DH = 192
NQ = H // 4
QR = 4 * DH
KT = D // 128
BW = 8
BDIL = 2
BDH = D // H
HIST = 16
NEG = -1000000000.0
EPS = 1e-5
NSLOT = 3
AHEAD = 2
LAG = 2
BCOUNT = (16, 4, 4, 2, 4, 6, 4, 4, 5)
SCHEDULE = "K1 K0 S3a-1 S3b-1 S3c-1 B S3d-1 K2 PVa-1 PVb-1 KPa KPb PVc-1 PVd-1 KPc B KPd OC-1 Q1 Q2 B Q0 V0 QKa QKb QKc QKd V1 S1a V2 OA-1 S2a S1c S1d VPa S1b B OB-1 S2d S2b VPc VPb OR-1 VPd S2c"


def _bf(x):
    return pltpu.bitcast(x, BF16)


def _u32(x):
    return pltpu.bitcast(x, U32)


def _dot(a, b):
    return lax.dot_general(a, b, (((1,), (0,)), ((), ())), preferred_element_type=F32)


def _dot_t(a, b):
    return lax.dot_general(a, b, (((1,), (1,)), ((), ())), preferred_element_type=F32)


def _layernorm(x):
    m = jnp.sum(x, axis=-1, keepdims=True) * (1.0 / D)
    c = x - m
    v = jnp.sum(c * c, axis=-1, keepdims=True) * (1.0 / D)
    return c * lax.rsqrt(v + EPS)


def _recip(l):
    r = pl.reciprocal(l, approx=True)
    return r * (2.0 - l * r)


def _add(a, b):
    return b if a is None else a if b is None else a + b


def _sub(a, b):
    return a if b is None else (-b if a is None else a - b)


def _lhs_combos(a11, a12, a21, a22):
    return [_add(a11, a22), _add(a21, a22), a11, a22, _add(a11, a12), _sub(a21, a11), _sub(a12, a22)]


def _rhs_combos(b11, b12, b21, b22):
    return [b11 + b22, b11, b12 - b22, b21 - b11, b22, b11 + b12, b21 + b22]


def _needed(live1, live2):
    return sorted(({0, 2, 3, 4, 6} if live1 else set()) | ({0, 1, 2, 3, 5} if live2 else set()))


def _recombine(m, live1=True, live2=True):
    top = (_add(_sub(_add(m[0], m[3]), m[4]), m[6]), _add(m[2], m[4])) if live1 else (None, None)
    bot = (_add(m[1], m[3]), _add(_add(_sub(m[0], m[1]), m[2]), m[5])) if live2 else (None, None)
    return top + bot


def _kernel(x_hbm, mem0_hbm, wqt_hbm, wkt_hbm, wvt_hbm, wo_hbm, bqkv_hbm, bwo_hbm,
            out_ref,
            xs, mem_s, x_s, h_s, stage, ws, wso, wsr, lhs,
            bst_qkv, bst_o, bqkv, bwo, kwin, vwin,
            sem_small, sem_a, sem_out):
    def seg_rows(seg):
        if isinstance(seg, int):
            return pl.ds(seg * SEG, SEG)
        return pl.ds(pl.multiple_of(seg * SEG, SEG), SEG)

    def a_copies(c):
        rows = pl.ds(c * QR, QR)
        return [pltpu.make_async_copy(src.at[rows, :], stage.at[c % NSLOT, w], sem_a.at[c, w])
                for w, src in enumerate((wqt_hbm, wkt_hbm, wvt_hbm, wo_hbm))]

    def input_layernorm(seg):
        r = seg_rows(seg)
        h_s[r, :] = _layernorm(xs[r, :].astype(F32))

    ri = lax.broadcasted_iota(jnp.int32, (D, D), 0)
    ci = lax.broadcasted_iota(jnp.int32, (D, D), 1)

    def permute_qkv(part):
        perm = jnp.where(ri == (ci & 31) * BDH + (ci >> 5), 1.0, 0.0).astype(BF16)
        wp = _dot(bst_qkv[:, part * D:(part + 1) * D], perm).astype(BF16)
        for j in range(KT):
            bqkv[part * KT + j] = _u32(wp[:, j * 128:(j + 1) * 128])

    def permute_wo():
        permt = jnp.where(ci == (ri & 31) * BDH + (ri >> 5), 1.0, 0.0).astype(BF16)
        wp = _dot(permt, bst_o[...]).astype(BF16)
        for j in range(KT):
            bwo[j] = _u32(wp[:, j * 128:(j + 1) * 128])

    def build_chunk(c):
        slot = c % NSLOT
        ei = lax.broadcasted_iota(jnp.int32, (128, 128), 0)
        ej = lax.broadcasted_iota(jnp.int32, (128, 128), 1)
        eye = jnp.where(ei == ej, 1.0, 0.0).astype(BF16)

        def qkv_block(w, _):
            for tt in range(3):
                idx = (w * NQ + c) * 3 + tt

                def tr(half, i):
                    r0 = (3 * half + tt) * 128
                    return _dot_t(eye, stage[slot, w, r0:r0 + 128, i * 128:(i + 1) * 128])

                for ii in range(2):
                    combos = _rhs_combos(tr(0, ii), tr(1, ii), tr(0, 2 + ii), tr(1, 2 + ii))
                    for i, cmb in enumerate(combos):
                        ws[idx, i * 128 + ii * 64:i * 128 + (ii + 1) * 64, :] = _u32(cmb.astype(BF16))
                ws[idx, 896:960, :] = _u32(tr(0, 4).astype(BF16))
                ws[idx, 960:1024, :] = _u32(tr(1, 4).astype(BF16))
            return 0
        lax.fori_loop(0, 3, qkv_block, 0)

        def o_block(n, _):
            npair = n // 3
            r = n % 3
            c1 = pl.ds(pl.multiple_of(npair * 256, 256), 128)
            c2 = pl.ds(pl.multiple_of(npair * 256 + 128, 128), 128)
            r1 = pl.ds(pl.multiple_of(r * 128, 128), 128)
            r2 = pl.ds(pl.multiple_of(384 + r * 128, 128), 128)
            combos = _rhs_combos(stage[slot, 3, r1, c1].astype(F32), stage[slot, 3, r1, c2].astype(F32),
                                 stage[slot, 3, r2, c1].astype(F32), stage[slot, 3, r2, c2].astype(F32))
            for i, cmb in enumerate(combos):
                wso[c * 2 + npair, pl.ds(pl.multiple_of(i * 192 + r * 64, 64), 64), :] = _u32(cmb.astype(BF16))
            return 0
        lax.fori_loop(0, 6, o_block, 0)
        wsr[c] = _u32(stage[slot, 3, :, 512:640])

    XH = 2 * SEG
    items = [
        ([pltpu.make_async_copy(x_hbm.at[pl.ds(0, XH), :], xs.at[pl.ds(0, XH), :], sem_small.at[0]),
          pltpu.make_async_copy(mem0_hbm, mem_s, sem_small.at[1])],
         [functools.partial(input_layernorm, 0)]),
        ([pltpu.make_async_copy(bqkv_hbm, bst_qkv, sem_small.at[2]),
          pltpu.make_async_copy(bwo_hbm, bst_o, sem_small.at[3])], [functools.partial(permute_qkv, 0)]),
    ]
    extra = [functools.partial(permute_qkv, 1), functools.partial(permute_qkv, 2), permute_wo]
    for c in range(NQ):
        work = [functools.partial(build_chunk, c)]
        if c < len(extra):
            work.append(extra[c])
        items.append((a_copies(c), work))
    items.append(([pltpu.make_async_copy(x_hbm.at[pl.ds(XH, S - XH), :], xs.at[pl.ds(XH, S - XH), :],
                                         sem_small.at[4])], []))

    def run_item(n):
        copies, work = items[n]
        if n + AHEAD < len(items):
            for cp in items[n + AHEAD][0]:
                cp.start()
        for cp in copies:
            cp.wait()
        for fn in work:
            fn()

    for copies, _ in items[:AHEAD]:
        for cp in copies:
            cp.start()

    kwin[...] = jnp.zeros(kwin.shape, F32)
    vwin[...] = jnp.zeros(vwin.shape, F32)
    x_s[pl.ds(S, SEG), :] = jnp.zeros((SEG, D), F32)
    xs[pl.ds(S, SEG), :] = jnp.zeros((SEG, D), BF16)
    run_item(0)
    run_item(1)

    mem0 = mem_s[...].astype(F32)

    lane = lax.broadcasted_iota(jnp.int32, (L, 128), 1)
    lo_half = lane < 64
    arow = lax.broadcasted_iota(jnp.int32, (L, 2 * L), 0)
    acol = lax.broadcasted_iota(jnp.int32, (L, 2 * L), 1)
    akey = jnp.where(acol < L, acol, acol - L)
    allowed = (arow >= SEG) | (akey >= SEG) | (akey <= arow)
    mask_e = allowed & (acol < L)
    mask_o = allowed & (acol >= L)
    a_scale = DH ** -0.5
    b_scale = BDH ** -0.5
    brow = lax.broadcasted_iota(jnp.int32, (SEG, 128), 0)

    def b_stages(s1, s2):
        live = [n for n, sg in enumerate((s1, s2)) if sg is not None]
        if not live:
            return
        segs = {n: (s1, s2)[n] for n in live}
        rows = {n: seg_rows(segs[n]) for n in live}
        off_of = {n: i * SEG for i, n in enumerate(live)}
        hn = jnp.concatenate([_layernorm(x_s[rows[n], :]) for n in live], axis=0)
        for n in live:
            kwin[n, 0:HIST, :] = kwin[n, SEG:SEG + HIST, :]
            vwin[n, 0:HIST, :] = vwin[n, SEG:SEG + HIST, :]
        yield
        q = []
        for j in range(KT):
            cols = slice(j * 128, (j + 1) * 128)
            k = _dot(hn, _bf(bqkv[KT + j]))
            for n in live:
                kwin[n, HIST:, cols] = k[off_of[n]:off_of[n] + SEG]
            yield
        for j in range(KT):
            q.append(_dot(hn, _bf(bqkv[j])))
            yield
        for j in range(KT):
            cols = slice(j * 128, (j + 1) * 128)
            v = _dot(hn, _bf(bqkv[2 * KT + j]))
            for n in live:
                vwin[n, HIST:, cols] = v[off_of[n]:off_of[n] + SEG]
            yield
        o = {n: [None] * KT for n in live}
        for n in live:
            pos = brow + segs[n] * SEG
            logits = []
            for w in range(BW):
                off = HIST - BDIL * w
                t = None
                for j in range(KT):
                    cols = slice(j * 128, (j + 1) * 128)
                    pj = q[j][off_of[n]:off_of[n] + SEG] * kwin[n, off:off + SEG, cols]
                    t = pj if t is None else t + pj
                t = t + pltpu.roll(t, 64, axis=1)
                t = t + pltpu.roll(t, 32, axis=1)
                logits.append(jnp.where(pos >= BDIL * w, t * b_scale, NEG))
                yield
            m = logits[0]
            for w in range(1, BW):
                m = jnp.maximum(m, logits[w])
            e = [jnp.exp(lg - m) for lg in logits]
            l = e[0]
            for w in range(1, BW):
                l = l + e[w]
            rl = _recip(l)
            a = [ew * rl for ew in e]
            yield
            for j in range(KT):
                cols = slice(j * 128, (j + 1) * 128)
                t = None
                for w in range(BW):
                    off = HIST - BDIL * w
                    pw = a[w] * vwin[n, off:off + SEG, cols]
                    t = pw if t is None else t + pw
                o[n][j] = t
                yield
        o = jnp.concatenate([jnp.concatenate(o[n], axis=1) for n in live], axis=0)
        y = []
        for j in range(KT):
            y.append(_dot(o, _bf(bwo[j])))
            yield
        y = jnp.concatenate(y, axis=1)
        for n in live:
            xn = x_s[rows[n], :] + y[off_of[n]:off_of[n] + SEG]
            x_s[rows[n], :] = xn
            if n == 0:
                h_s[rows[n], :] = _layernorm(xn)
            else:
                xs[rows[n], :] = xn.astype(BF16)
        yield

    def advance(gen, n):
        for _ in range(n):
            next(gen, None)

    def a_layers(h1, h2, bgen, weights_ready=None):
        live1, live2 = h1 is not None, h2 is not None
        need = _needed(live1, live2)
        live_inst = ([0, 1] if live1 else []) + ([2, 3] if live2 else [])
        inst = [dict() for _ in range(4 * NQ)]
        acc_m = [[None] * 7, [None] * 7]
        acc_r = [None]
        blk = lambda h, j: None if h is None else h[:, 256 * j:256 * (j + 1)]
        have = {}
        for i, cmb in enumerate(_lhs_combos(blk(h1, 0), blk(h1, 1), blk(h2, 0), blk(h2, 1))):
            if i in need and cmb is not None:
                lhs[i] = cmb
                have[i] = True
        rem = jnp.concatenate([h[:, 512:] for h in (h1, h2) if h is not None], axis=0)

        def split_rows(r):
            if live1 and live2:
                return r[:L], r[L:]
            return (r, None) if live1 else (None, r)

        def pack_kv(t):
            ac = jnp.concatenate([t[0], t[2]], axis=0).astype(BF16)
            bb = jnp.concatenate([jnp.where(lo_half, t[1], 0.0),
                                  jnp.where(lo_half, 0.0, t[1])], axis=0).astype(BF16)
            return ac, bb

        def run(op, qd):
            if op[0] in "KQV" and op[1] in "012":
                tt = int(op[1])
                idx = ("QKV".index(op[0]) * NQ + qd) * 3 + tt
                mi = [_dot(lhs[i], _bf(ws[idx, 128 * i:128 * (i + 1), :])) if i in have else None
                      for i in range(7)]
                r1 = split_rows(_dot(rem, _bf(ws[idx, 896:960, :])))
                r2 = split_rows(_dot(rem, _bf(ws[idx, 960:1024, :])))
                c = _recombine(mi, live1, live2)
                for n, r in enumerate((r1[0], r2[0], r1[1], r2[1])):
                    if n in live_inst:
                        inst[qd * 4 + n].setdefault(op[0], {})[tt] = c[n] + r
                return
            if op == "OC":
                o = [inst[qd * 4 + n].pop("o") if n in live_inst else None for n in range(4)]
                inst[qd * 4]["oc"] = [cmb if i in need else None for i, cmb in enumerate(_lhs_combos(*o))]
                inst[qd * 4]["orem"] = jnp.concatenate(
                    [jnp.concatenate([o[2 * n], o[2 * n + 1]], axis=1) for n in range(2)
                     if o[2 * n] is not None], axis=0)
                return
            if op in ("OA", "OB"):
                npair = "AB".index(op[1])
                for i, cmb in enumerate(inst[qd * 4]["oc"]):
                    if cmb is not None:
                        part = _dot(cmb, _bf(wso[qd * 2 + npair, 192 * i:192 * (i + 1), :]))
                        acc_m[npair][i] = _add(acc_m[npair][i], part)
                return
            if op == "OR":
                part = _dot(inst[qd * 4].pop("orem"), _bf(wsr[qd]))
                acc_r[0] = _add(acc_r[0], part)
                return
            if "abcd".index(op[2]) not in live_inst:
                return
            d = inst[qd * 4 + "abcd".index(op[2])]
            op = op[:2]
            if op == "KP":
                d["kp"] = pack_kv(d.pop("K"))
            elif op == "VP":
                d["vp"] = pack_kv(d.pop("V"))
            elif op == "QK":
                q = d.pop("Q")
                k_ac, k_b = d.pop("kp")
                d["sc"] = (_dot_t(jnp.concatenate([q[0], q[2]], axis=0), k_ac), _dot_t(q[1], k_b))
            elif op == "S1":
                s_ac, s_b = d.pop("sc")
                s_e = jnp.where(mask_e, (s_ac[:L] + s_b) * a_scale, NEG)
                s_o = jnp.where(mask_o, (s_ac[L:] + s_b) * a_scale, NEG)
                d["mx"] = [(s, jnp.max(s, axis=-1, keepdims=True)) for s in (s_e, s_o)]
            elif op == "S2":
                es = [jnp.exp(s - m) for s, m in d.pop("mx")]
                d["pr"] = [(e, jnp.sum(e, axis=-1, keepdims=True)) for e in es]
            elif op == "S3":
                d["p"] = [e * _recip(l) for e, l in d.pop("pr")]
            elif op == "PV":
                p_e, p_o = d.pop("p")
                v_ac, v_b = d.pop("vp")
                o_ac = _dot(jnp.concatenate([p_e, p_o], axis=0), v_ac)
                o_b = _dot(p_e + p_o, v_b)
                d["o"] = jnp.concatenate([o_ac[:L], o_b, o_ac[L:]], axis=1)
            else:
                raise ValueError(op)

        toks = SCHEDULE.split()
        maxlag = max(int(t.partition("-")[2] or 0) for t in toks)
        nb = toks.count("B")
        for i in range(NQ + maxlag):
            if weights_ready is not None and i < NQ:
                weights_ready(i)
            bi = 0
            for tok in toks:
                if tok == "B":
                    n = BCOUNT[i] if i < len(BCOUNT) else 0
                    advance(bgen, (n * (bi + 1)) // nb - (n * bi) // nb)
                    bi += 1
                    continue
                op, _, lag = tok.partition("-")
                qd = i - int(lag or 0)
                if 0 <= qd < NQ:
                    run(op, qd)
        blocks = [_recombine(acc_m[npair], live1, live2) for npair in range(2)]
        r4 = split_rows(acc_r[0])
        y1 = y2 = None
        if live1:
            y1 = jnp.concatenate([blocks[0][0], blocks[0][1], blocks[1][0], blocks[1][1], r4[0]], axis=1)
        if live2:
            y2 = jnp.concatenate([blocks[0][2], blocks[0][3], blocks[1][2], blocks[1][3], r4[1]], axis=1)
        return y1, y2

    def out_copy(seg):
        r = seg_rows(seg)
        return pltpu.make_async_copy(xs.at[r, :], out_ref.at[r, :], sem_out.at[0])

    def step(t, carry, first=False):
        mem1, mem2 = carry
        static = isinstance(t, int)
        valid = lambda sg: sg if (not static or 0 <= sg < NSEG) else None
        s1, s2, sb1, sb2 = valid(t), valid(t - LAG), valid(t - 1), valid(t - LAG - 1)
        if not static:
            sb2 = jnp.where(sb2 < 0, NSEG, sb2)
        h1 = None if s1 is None else jnp.concatenate([h_s[seg_rows(s1), :], mem1], axis=0)
        h2 = None if s2 is None else jnp.concatenate([h_s[seg_rows(s2), :], mem2], axis=0)
        bgen = b_stages(sb1, sb2)
        if s1 is not None and (not static or s1 + 1 < NSEG):
            input_layernorm(s1 + 1)
        y1, y2 = a_layers(h1, h2, bgen, (lambda c: run_item(2 + c)) if first else None)
        advance(bgen, 1000)
        if s1 is not None:
            x_s[seg_rows(s1), :] = xs[seg_rows(s1), :].astype(F32) + y1[:SEG]
            mem1 = y1[SEG:]
        if s2 is not None:
            x_s[seg_rows(s2), :] = x_s[seg_rows(s2), :] + y2[:SEG]
            mem2 = y2[SEG:]
        if static:
            if sb2 is not None:
                out_copy(sb2).start()
        else:
            @pl.when(t - LAG - 1 >= 0)
            def _():
                out_copy(t - LAG - 1).start()
        return mem1, mem2

    carry = step(0, (mem0, mem0), first=True)
    run_item(len(items) - 1)
    for t in range(1, LAG):
        carry = step(t, carry)
    carry = lax.fori_loop(LAG, NSEG, step, carry)
    for t in range(NSEG, NSEG + LAG):
        carry = step(t, carry)
    advance(b_stages(None, NSEG - 1), 1000)
    out_copy(NSEG - 1).start()

    def wait_out(i, _):
        out_copy(i).wait()
        return 0
    lax.fori_loop(0, NSEG, wait_out, 0)


@functools.partial(jax.jit, static_argnames=("A_seg_len",))
def pallas_interleave_layers__memory_aug_recurrent_mem_tr__sliding_local_dilated__prompt_kernel(
    A_x, A_mem0, A_Wq, A_Wk, A_Wv, A_Wo, A_seg_len, B_x, B_wqkv, B_wo,
):
    del B_x
    assert int(A_seg_len) == SEG
    assert A_x.shape == (1, S, D) and A_mem0.shape == (1, M, D)
    assert A_Wq.shape == (D, H, DH) and A_Wo.shape == (H, DH, D)

    def wt(w):
        return jnp.transpose(w, (1, 2, 0)).reshape(H * DH, D)

    any_spec = pl.BlockSpec(memory_space=pl.ANY)
    out = pl.pallas_call(
        _kernel,
        out_shape=jax.ShapeDtypeStruct((S, D), BF16),
        in_specs=[any_spec] * 8,
        out_specs=any_spec,
        scratch_shapes=[
            pltpu.VMEM((S + SEG, D), BF16),
            pltpu.VMEM((M, D), BF16),
            pltpu.VMEM((S + SEG, D), F32),
            pltpu.VMEM((S + SEG, D), F32),
            pltpu.VMEM((NSLOT, 4, QR, D), BF16),
            pltpu.VMEM((3 * NQ * 3, 1024, 128), U32),
            pltpu.VMEM((NQ * 2, 7 * 192, 128), U32),
            pltpu.VMEM((NQ, QR // 2, 128), U32),
            pltpu.VMEM((7, L, 256), F32),
            pltpu.VMEM((D, 3 * D), BF16),
            pltpu.VMEM((D, D), BF16),
            pltpu.VMEM((3 * KT, D // 2, 128), U32),
            pltpu.VMEM((KT, D // 2, 128), U32),
            pltpu.VMEM((2, HIST + SEG, D), F32),
            pltpu.VMEM((2, HIST + SEG, D), F32),
            pltpu.SemaphoreType.DMA((5,)),
            pltpu.SemaphoreType.DMA((NQ, 4)),
            pltpu.SemaphoreType.DMA((1,)),
        ],
        compiler_params=pltpu.CompilerParams(vmem_limit_bytes=120 * 1024 * 1024),
        name="interleaved_rmt_dilated",
    )(A_x.reshape(S, D), A_mem0.reshape(M, D), wt(A_Wq), wt(A_Wk), wt(A_Wv),
      A_Wo.reshape(H * DH, D), B_wqkv, B_wo)
    return out.reshape(1, S, D)
```

```python
import functools

import jax
import jax.numpy as jnp
from jax import lax
import jax.experimental.pallas as pl
import jax.experimental.pallas.tpu as pltpu

F32 = jnp.float32
BF16 = jnp.bfloat16
U32 = jnp.uint32

S = 2048
D = 640
SEG = 32
M = 8
NSEG = S // SEG
L = SEG + M
H = 32
DH = 192
NP = H // 2
PR = 2 * DH
NCH = NP // 2
CR = 2 * PR
KT = D // 128
BW = 8
BDIL = 2
BDH = D // H
HIST = 16
NEG = -1000000000.0
EPS = 1e-5
NSLOT = 3
AHEAD = 2
LAG = 2
BCOUNT = (10, 8, 2, 2, 2, 4, 2, 2, 4, 0, 0, 0, 2, 4, 2, 2, 3)
SCHEDULE = "S3b-1 K0 K1 K2 Q0 K3 S3a-1 B PVa-1 K4 Q1 PVb-1 KPb Q2 Q3 B Q4 B KPa O0-1 V0 QKa O1-1 V1 QKb S1b V2 V3 O2-1 V4 S2b O3-1 S1a O4-1 S2a VPa VPb"


def _bf(x):
    return pltpu.bitcast(x, BF16)


def _u32(x):
    return pltpu.bitcast(x, U32)


def _dot(a, b):
    return lax.dot_general(a, b, (((1,), (0,)), ((), ())), preferred_element_type=F32)


def _dot_t(a, b):
    return lax.dot_general(a, b, (((1,), (1,)), ((), ())), preferred_element_type=F32)


def _layernorm(x):
    m = jnp.sum(x, axis=-1, keepdims=True) * (1.0 / D)
    c = x - m
    v = jnp.sum(c * c, axis=-1, keepdims=True) * (1.0 / D)
    return c * lax.rsqrt(v + EPS)


def _recip(l):
    r = pl.reciprocal(l, approx=True)
    return r * (2.0 - l * r)


_U = (
    ( 0,  0, -1,  0,  0,  0,  0,  1,  0,  0),
    ( 1,  0,  0,  0, -1, -1,  0,  0,  0,  1),
    ( 0,  0,  0,  0,  0,  0, -1,  0,  0,  0),
    ( 0,  0,  0,  1,  0,  0,  0,  0, -1,  0),
    ( 0, -1,  0,  1,  0,  0,  0,  0,  0,  0),
    ( 0,  0, -1,  0,  0,  0,  0,  0,  0,  0),
    ( 0,  0,  0,  1,  1,  0,  0,  0, -1, -1),
    (-1,  0,  0,  0,  1,  1,  0,  0,  0,  0),
    ( 0,  0,  0,  0,  0, -1,  0,  0,  0,  0),
    ( 0,  1,  0,  0,  0,  0, -1,  0,  0,  0),
    ( 0,  0,  0, -1,  0,  0,  1,  0,  0,  0),
    (-1,  0, -1,  0,  0,  0,  0,  0,  0,  0),
    ( 1,  0,  0,  0,  0, -1,  0,  0,  0,  0),
    ( 0,  0,  0,  0,  0,  0,  1,  0, -1,  0),
    ( 0,  0,  0,  0,  0,  1,  0,  1,  0,  0),
    ( 0,  0,  0,  0, -1,  0,  0,  0,  0,  0),
    ( 0,  0,  1,  0,  0,  0, -1,  0,  0,  0),
    ( 0,  0,  0, -1,  0,  0,  0,  0,  1,  1),
    ( 0,  0,  0,  0,  0,  0,  0,  0, -1, -1),
    ( 0,  0,  0,  0,  0,  0,  0,  0,  0, -1),
    ( 0,  0,  0,  0,  0,  0, -1,  1,  0,  0),
    ( 0, -1,  1,  0,  0,  0,  0,  0,  0,  0),
    ( 0,  0, -1,  0,  0, -1,  0,  0,  0,  0),
    ( 0,  0,  0,  1,  0,  0,  0,  0,  0,  0),
    ( 1,  0,  0,  0, -1,  0,  0,  0,  0,  0),
)
_V = (
    ( 0,  0,  0,  0,  0,  0,  1,  0,  1,  0,  0,  0,  0,  0,  0),
    ( 0,  0,  0,  0,  0,  0,  0,  0,  0,  0,  0,  0,  1,  0, -1),
    ( 0,  0,  0,  0,  0, -1,  0,  0, -1,  1,  0, -1,  0,  0,  0),
    ( 0,  0,  0,  0,  0,  0,  0,  0,  0, -1, -1,  1,  0,  1,  0),
    ( 0,  0,  0,  1,  1,  0,  0,  0,  0,  0,  0,  0,  0,  0,  0),
    ( 0,  1,  0,  1,  0,  0,  0, -1,  0,  0,  0,  0,  0,  0,  0),
    ( 0,  0,  0,  0,  0,  0,  0,  0,  0,  0,  0,  0,  0,  1,  0),
    ( 0,  0, -1,  0,  0,  0,  0,  0,  0,  0,  0,  0,  1,  0, -1),
    ( 1,  1,  0,  0,  0,  0, -1, -1,  0,  0,  0,  0,  0,  0,  0),
    ( 0,  0,  0,  0,  1, -1,  0,  0,  0,  0,  0,  0,  0,  0,  0),
    ( 0,  0,  0,  1,  1,  0,  0,  0,  0, -1,  0,  1,  0,  0,  0),
    ( 0, -1,  0,  0,  0,  0,  0,  0,  0,  0,  0,  0,  0,  0,  0),
    ( 1,  0, -1,  0,  0,  0,  0,  0,  0,  0,  0,  0,  1,  0, -1),
    ( 0,  0,  0,  0,  0,  0,  0,  0,  0,  1,  0, -1,  0,  0,  0),
    ( 0,  0,  0,  0,  0,  0,  1,  1,  0,  0,  0,  0,  0,  0,  0),
    ( 0,  0,  1,  0,  0,  0,  0,  0,  0,  0,  0,  0,  0, -1,  1),
    ( 0,  0,  0, -1,  0,  0,  0,  0,  1,  0,  0,  0,  0,  0,  0),
    ( 0,  0,  0,  0,  0,  0,  0,  0,  0, -1,  0,  0,  0,  1,  0),
    ( 0,  0,  0,  0,  0,  0,  0,  0,  0,  1,  0,  0,  0,  0,  0),
    ( 0,  0,  0,  0,  0,  0,  0,  0,  0, -1,  0,  0,  1,  0,  0),
    ( 0,  0,  0,  0,  0,  0,  0,  0,  1,  0,  0,  0,  0,  0,  0),
    ( 0,  0,  0, -1,  0,  0,  0,  0,  0,  0,  0,  0,  0,  0,  0),
    ( 0,  1,  0,  0,  0,  0, -1, -1,  0,  0,  0,  0,  0,  0,  0),
    ( 0,  0,  0, -1, -1,  0,  0,  0,  0,  1, -1,  0,  0,  0,  0),
    ( 0,  0,  1,  0,  0,  0,  0,  0,  0,  0,  0,  0,  0,  0,  0),
)
_W = (
    ( 0,  0,  0,  1, -1,  0),
    ( 0,  0,  0,  0,  0, -1),
    ( 0,  0,  1,  0,  0,  1),
    ( 0,  0,  0,  0,  1,  0),
    ( 0, -1, -1,  0,  0,  0),
    (-1,  1,  0, -1,  1,  0),
    ( 1,  1,  1,  0,  0,  0),
    ( 1,  0,  0,  0,  0, -1),
    (-1,  0,  0, -1,  0,  0),
    ( 0,  0, -1,  0,  0,  0),
    ( 0,  0, -1,  0,  1,  0),
    ( 0,  1,  0,  0,  0,  0),
    ( 1,  0,  0,  0,  0,  0),
    ( 0,  0,  0,  0,  1,  1),
    ( 0,  0,  0,  0,  1,  0),
    (-1,  0, -1,  0,  0,  0),
    ( 0,  0,  1,  1, -1,  0),
    ( 1,  1,  1,  0,  1,  0),
    (-1, -1, -1, -1, -1, -1),
    ( 0,  0,  0, -1,  0, -1),
    ( 0,  0,  0, -1,  1,  1),
    ( 1, -1, -1,  0,  0,  0),
    ( 1,  0,  0,  1, -1,  0),
    ( 0, -1,  0,  0, -1,  0),
    ( 0,  0,  1,  0,  0,  1),
)
NR = len(_U)
NPART = 5


def _comb(coefs, blocks):
    acc = None
    for c, blk in zip(coefs, blocks):
        if c == 0 or blk is None:
            continue
        if acc is None:
            acc = blk if c > 0 else -blk
        else:
            acc = acc + blk if c > 0 else acc - blk
    return acc


def _needed(live):
    return [r for r in range(NR)
            if any(_U[r][5 * m + j] for m in live for j in range(5))
            and any(_W[r][3 * m + k] for m in live for k in range(3))]


def _parts(seq):
    n = len(seq)
    return [seq[(n * i) // NPART:(n * (i + 1)) // NPART] for i in range(NPART)]


def _kernel(x_hbm, mem0_hbm, wqt_hbm, wkt_hbm, wvt_hbm, wo_hbm, bqkv_hbm, bwo_hbm,
            out_ref,
            xs, mem_s, x_s, h_s, stage, ws, wso, lhs, accm,
            bst_qkv, bst_o, bqkv, bwo, kwin, vwin,
            sem_small, sem_a, sem_out):
    def seg_rows(seg):
        if isinstance(seg, int):
            return pl.ds(seg * SEG, SEG)
        return pl.ds(pl.multiple_of(seg * SEG, SEG), SEG)

    def a_copies(c):
        rows = pl.ds(c * CR, CR)
        return [pltpu.make_async_copy(src.at[rows, :], stage.at[c % NSLOT, w], sem_a.at[c, w])
                for w, src in enumerate((wqt_hbm, wkt_hbm, wvt_hbm, wo_hbm))]

    def input_layernorm(seg):
        r = seg_rows(seg)
        h_s[r, :] = _layernorm(xs[r, :].astype(F32))

    ri = lax.broadcasted_iota(jnp.int32, (D, D), 0)
    ci = lax.broadcasted_iota(jnp.int32, (D, D), 1)

    def permute_qkv(part):
        perm = jnp.where(ri == (ci & 31) * BDH + (ci >> 5), 1.0, 0.0).astype(BF16)
        wp = _dot(bst_qkv[:, part * D:(part + 1) * D], perm).astype(BF16)
        for j in range(KT):
            bqkv[part * KT + j] = _u32(wp[:, j * 128:(j + 1) * 128])

    def permute_wo():
        permt = jnp.where(ci == (ri & 31) * BDH + (ri >> 5), 1.0, 0.0).astype(BF16)
        wp = _dot(permt, bst_o[...]).astype(BF16)
        for j in range(KT):
            bwo[j] = _u32(wp[:, j * 128:(j + 1) * 128])

    def build_chunk(c):
        slot = c % NSLOT
        ei = lax.broadcasted_iota(jnp.int32, (128, 128), 0)
        ej = lax.broadcasted_iota(jnp.int32, (128, 128), 1)
        eye = jnp.where(ei == ej, 1.0, 0.0).astype(BF16)

        def qkv_block(n, _):
            w = n // 2
            pp = n % 2
            g = w * NP + 2 * c + pp
            tiles = []
            for j in range(KT):
                for k in range(3):
                    r = pl.ds(pl.multiple_of(pp * PR + k * 128, 128), 128)
                    tiles.append(_dot_t(eye, stage[slot, w, r, j * 128:(j + 1) * 128]))
            for r in range(NR):
                ws[g, 64 * r:64 * (r + 1), :] = _u32(_comb(_V[r], tiles).astype(BF16))
            return 0
        lax.fori_loop(0, 6, qkv_block, 0)

        def o_block(pp, _):
            tiles = []
            for j in range(KT):
                for k in range(3):
                    r = pl.ds(pl.multiple_of(pp * PR + k * 128, 128), 128)
                    tiles.append(stage[slot, 3, r, j * 128:(j + 1) * 128].astype(F32))
            for r in range(NR):
                wso[2 * c + pp, 64 * r:64 * (r + 1), :] = _u32(_comb(_V[r], tiles).astype(BF16))
            return 0
        lax.fori_loop(0, 2, o_block, 0)

    XH = 2 * SEG
    items = [
        ([pltpu.make_async_copy(x_hbm.at[pl.ds(0, XH), :], xs.at[pl.ds(0, XH), :], sem_small.at[0]),
          pltpu.make_async_copy(mem0_hbm, mem_s, sem_small.at[1])],
         [functools.partial(input_layernorm, 0)]),
        ([pltpu.make_async_copy(bqkv_hbm, bst_qkv, sem_small.at[2]),
          pltpu.make_async_copy(bwo_hbm, bst_o, sem_small.at[3])], [functools.partial(permute_qkv, 0)]),
    ]
    extra = [functools.partial(permute_qkv, 1), functools.partial(permute_qkv, 2), permute_wo]
    for c in range(NCH):
        work = [functools.partial(build_chunk, c)]
        if c < len(extra):
            work.append(extra[c])
        items.append((a_copies(c), work))
    items.append(([pltpu.make_async_copy(x_hbm.at[pl.ds(XH, S - XH), :], xs.at[pl.ds(XH, S - XH), :],
                                         sem_small.at[4])], []))

    def run_item(n):
        copies, work = items[n]
        if n + AHEAD < len(items):
            for cp in items[n + AHEAD][0]:
                cp.start()
        for cp in copies:
            cp.wait()
        for fn in work:
            fn()

    for copies, _ in items[:AHEAD]:
        for cp in copies:
            cp.start()

    kwin[...] = jnp.zeros(kwin.shape, F32)
    vwin[...] = jnp.zeros(vwin.shape, F32)
    x_s[pl.ds(S, SEG), :] = jnp.zeros((SEG, D), F32)
    xs[pl.ds(S, SEG), :] = jnp.zeros((SEG, D), BF16)
    run_item(0)
    run_item(1)

    mem0 = mem_s[...].astype(F32)

    lane = lax.broadcasted_iota(jnp.int32, (L, 128), 1)
    lo_half = lane < 64
    arow = lax.broadcasted_iota(jnp.int32, (L, 2 * L), 0)
    acol = lax.broadcasted_iota(jnp.int32, (L, 2 * L), 1)
    akey = jnp.where(acol < L, acol, acol - L)
    allowed = (arow >= SEG) | (akey >= SEG) | (akey <= arow)
    mask_e = allowed & (acol < L)
    mask_o = allowed & (acol >= L)
    a_scale = DH ** -0.5
    b_scale = BDH ** -0.5
    brow = lax.broadcasted_iota(jnp.int32, (SEG, 128), 0)

    def b_stages(s1, s2):
        live = [n for n, sg in enumerate((s1, s2)) if sg is not None]
        if not live:
            return
        segs = {n: (s1, s2)[n] for n in live}
        rows = {n: seg_rows(segs[n]) for n in live}
        off_of = {n: i * SEG for i, n in enumerate(live)}
        hn = jnp.concatenate([_layernorm(x_s[rows[n], :]) for n in live], axis=0)
        for n in live:
            kwin[n, 0:HIST, :] = kwin[n, SEG:SEG + HIST, :]
            vwin[n, 0:HIST, :] = vwin[n, SEG:SEG + HIST, :]
        yield
        q = []
        for j in range(KT):
            cols = slice(j * 128, (j + 1) * 128)
            k = _dot(hn, _bf(bqkv[KT + j]))
            for n in live:
                kwin[n, HIST:, cols] = k[off_of[n]:off_of[n] + SEG]
            yield
        for j in range(KT):
            q.append(_dot(hn, _bf(bqkv[j])))
            yield
        for j in range(KT):
            cols = slice(j * 128, (j + 1) * 128)
            v = _dot(hn, _bf(bqkv[2 * KT + j]))
            for n in live:
                vwin[n, HIST:, cols] = v[off_of[n]:off_of[n] + SEG]
            yield
        o = {n: [None] * KT for n in live}
        for n in live:
            pos = brow + segs[n] * SEG
            logits = []
            for w in range(BW):
                off = HIST - BDIL * w
                t = None
                for j in range(KT):
                    cols = slice(j * 128, (j + 1) * 128)
                    pj = q[j][off_of[n]:off_of[n] + SEG] * kwin[n, off:off + SEG, cols]
                    t = pj if t is None else t + pj
                t = t + pltpu.roll(t, 64, axis=1)
                t = t + pltpu.roll(t, 32, axis=1)
                logits.append(jnp.where(pos >= BDIL * w, t * b_scale, NEG))
                yield
            m = logits[0]
            for w in range(1, BW):
                m = jnp.maximum(m, logits[w])
            e = [jnp.exp(lg - m) for lg in logits]
            l = e[0]
            for w in range(1, BW):
                l = l + e[w]
            rl = _recip(l)
            a = [ew * rl for ew in e]
            yield
            for j in range(KT):
                cols = slice(j * 128, (j + 1) * 128)
                t = None
                for w in range(BW):
                    off = HIST - BDIL * w
                    pw = a[w] * vwin[n, off:off + SEG, cols]
                    t = pw if t is None else t + pw
                o[n][j] = t
                yield
        o = jnp.concatenate([jnp.concatenate(o[n], axis=1) for n in live], axis=0)
        y = []
        for j in range(KT):
            y.append(_dot(o, _bf(bwo[j])))
            yield
        y = jnp.concatenate(y, axis=1)
        for n in live:
            xn = x_s[rows[n], :] + y[off_of[n]:off_of[n] + SEG]
            x_s[rows[n], :] = xn
            if n == 0:
                h_s[rows[n], :] = _layernorm(xn)
            else:
                xs[rows[n], :] = xn.astype(BF16)
        yield

    def advance(gen, n):
        for _ in range(n):
            next(gen, None)

    def a_layers(h1, h2, bgen, weights_ready=None):
        live = [m for m, h in enumerate((h1, h2)) if h is not None]
        need = _needed(live)
        parts = _parts(need)
        inst = [dict() for _ in range(2 * NP)]
        hb = [None if h is None else h[:, 128 * j:128 * (j + 1)] for h in (h1, h2) for j in range(KT)]
        for r in need:
            lhs[r] = _comb(_U[r], hb)
        yb = [None] * (2 * KT)

        def pack_kv(t):
            ac = jnp.concatenate([t[0], t[2]], axis=0).astype(BF16)
            bb = jnp.concatenate([jnp.where(lo_half, t[1], 0.0),
                                  jnp.where(lo_half, 0.0, t[1])], axis=0).astype(BF16)
            return ac, bb

        def run(op, p):
            if op[0] in "KQV" and op[1].isdigit():
                g = "QKV".index(op[0]) * NP + p
                c = inst[2 * p].setdefault("c" + op[0], [None] * 6)
                for r in parts[int(op[1])]:
                    mr = _dot(lhs[r], _bf(ws[g, 64 * r:64 * (r + 1), :]))
                    for o in range(6):
                        if o // 3 in live and _W[r][o]:
                            c[o] = _comb((1, _W[r][o]), (c[o], mr))
                if int(op[1]) == NPART - 1:
                    for m in live:
                        inst[2 * p + m][op[0]] = c[3 * m:3 * m + 3]
                    del inst[2 * p]["c" + op[0]]
                return
            if op[0] == "O" and op[1].isdigit():
                d = inst[2 * p]
                if "ob" not in d:
                    d["ob"] = [inst[2 * p + m].pop("o") if m in live else [None] * 3 for m in range(2)]
                    d["ob"] = d["ob"][0] + d["ob"][1]
                for r in parts[int(op[1])]:
                    mr = _dot(_comb(_W[r], d["ob"]), _bf(wso[p, 64 * r:64 * (r + 1), :]))
                    if p == 0:
                        accm[r] = mr
                    elif p < NP - 1:
                        accm[r] = accm[r] + mr
                    else:
                        mr = accm[r] + mr
                        for a in range(2 * KT):
                            if a // KT in live and _U[r][a]:
                                yb[a] = _comb((1, _U[r][a]), (yb[a], mr))
                return
            if "ab".index(op[2]) not in live:
                return
            d = inst[2 * p + "ab".index(op[2])]
            op = op[:2]
            if op == "KP":
                d["kp"] = pack_kv(d.pop("K"))
            elif op == "VP":
                d["vp"] = pack_kv(d.pop("V"))
            elif op == "QK":
                q = d.pop("Q")
                k_ac, k_b = d.pop("kp")
                d["sc"] = (_dot_t(jnp.concatenate([q[0], q[2]], axis=0), k_ac), _dot_t(q[1], k_b))
            elif op == "S1":
                s_ac, s_b = d.pop("sc")
                s_e = jnp.where(mask_e, (s_ac[:L] + s_b) * a_scale, NEG)
                s_o = jnp.where(mask_o, (s_ac[L:] + s_b) * a_scale, NEG)
                d["mx"] = [(s, jnp.max(s, axis=-1, keepdims=True)) for s in (s_e, s_o)]
            elif op == "S2":
                es = [jnp.exp(s - m) for s, m in d.pop("mx")]
                d["pr"] = [(e, jnp.sum(e, axis=-1, keepdims=True)) for e in es]
            elif op == "S3":
                d["p"] = [e * _recip(l) for e, l in d.pop("pr")]
            elif op == "PV":
                p_e, p_o = d.pop("p")
                v_ac, v_b = d.pop("vp")
                o_ac = _dot(jnp.concatenate([p_e, p_o], axis=0), v_ac)
                o_b = _dot(p_e + p_o, v_b)
                d["o"] = [o_ac[:L], o_b, o_ac[L:]]
            else:
                raise ValueError(op)

        toks = SCHEDULE.split()
        maxlag = max(int(t.partition("-")[2] or 0) for t in toks)
        nb = toks.count("B")
        for i in range(NP + maxlag):
            if weights_ready is not None and i < NP and i % 2 == 0:
                weights_ready(i // 2)
            bi = 0
            for tok in toks:
                if tok == "B":
                    n = BCOUNT[i] if i < len(BCOUNT) else 0
                    advance(bgen, (n * (bi + 1)) // nb - (n * bi) // nb)
                    bi += 1
                    continue
                op, _, lag = tok.partition("-")
                p = i - int(lag or 0)
                if 0 <= p < NP:
                    run(op, p)
        return [jnp.concatenate(yb[KT * m:KT * (m + 1)], axis=1) if m in live else None for m in range(2)]

    def out_copy(seg):
        r = seg_rows(seg)
        return pltpu.make_async_copy(xs.at[r, :], out_ref.at[r, :], sem_out.at[0])

    def step(t, carry, first=False):
        mem1, mem2 = carry
        static = isinstance(t, int)
        valid = lambda sg: sg if (not static or 0 <= sg < NSEG) else None
        s1, s2, sb1, sb2 = valid(t), valid(t - LAG), valid(t - 1), valid(t - LAG - 1)
        if not static:
            sb2 = jnp.where(sb2 < 0, NSEG, sb2)
        h1 = None if s1 is None else jnp.concatenate([h_s[seg_rows(s1), :], mem1], axis=0)
        h2 = None if s2 is None else jnp.concatenate([h_s[seg_rows(s2), :], mem2], axis=0)
        bgen = b_stages(sb1, sb2)
        if s1 is not None and (not static or s1 + 1 < NSEG):
            input_layernorm(s1 + 1)
        y1, y2 = a_layers(h1, h2, bgen, (lambda c: run_item(2 + c)) if first else None)
        advance(bgen, 1000)
        if s1 is not None:
            x_s[seg_rows(s1), :] = xs[seg_rows(s1), :].astype(F32) + y1[:SEG]
            mem1 = y1[SEG:]
        if s2 is not None:
            x_s[seg_rows(s2), :] = x_s[seg_rows(s2), :] + y2[:SEG]
            mem2 = y2[SEG:]
        if static:
            if sb2 is not None:
                out_copy(sb2).start()
        else:
            @pl.when(t - LAG - 1 >= 0)
            def _():
                out_copy(t - LAG - 1).start()
        return mem1, mem2

    carry = step(0, (mem0, mem0), first=True)
    run_item(len(items) - 1)
    for t in range(1, LAG):
        carry = step(t, carry)
    carry = lax.fori_loop(LAG, NSEG, step, carry)
    for t in range(NSEG, NSEG + LAG):
        carry = step(t, carry)
    advance(b_stages(None, NSEG - 1), 1000)
    out_copy(NSEG - 1).start()

    def wait_out(i, _):
        out_copy(i).wait()
        return 0
    lax.fori_loop(0, NSEG, wait_out, 0)


@functools.partial(jax.jit, static_argnames=("A_seg_len",))
def pallas_interleave_layers__memory_aug_recurrent_mem_tr__sliding_local_dilated__prompt_kernel(
    A_x, A_mem0, A_Wq, A_Wk, A_Wv, A_Wo, A_seg_len, B_x, B_wqkv, B_wo,
):
    del B_x
    assert int(A_seg_len) == SEG
    assert A_x.shape == (1, S, D) and A_mem0.shape == (1, M, D)
    assert A_Wq.shape == (D, H, DH) and A_Wo.shape == (H, DH, D)

    def wt(w):
        return jnp.transpose(w, (1, 2, 0)).reshape(H * DH, D)

    any_spec = pl.BlockSpec(memory_space=pl.ANY)
    out = pl.pallas_call(
        _kernel,
        out_shape=jax.ShapeDtypeStruct((S, D), BF16),
        in_specs=[any_spec] * 8,
        out_specs=any_spec,
        scratch_shapes=[
            pltpu.VMEM((S + SEG, D), BF16),
            pltpu.VMEM((M, D), BF16),
            pltpu.VMEM((S + SEG, D), F32),
            pltpu.VMEM((S + SEG, D), F32),
            pltpu.VMEM((NSLOT, 4, CR, D), BF16),
            pltpu.VMEM((3 * NP, NR * 64, 128), U32),
            pltpu.VMEM((NP, NR * 64, 128), U32),
            pltpu.VMEM((NR, L, 128), F32),
            pltpu.VMEM((NR, L, 128), F32),
            pltpu.VMEM((D, 3 * D), BF16),
            pltpu.VMEM((D, D), BF16),
            pltpu.VMEM((3 * KT, D // 2, 128), U32),
            pltpu.VMEM((KT, D // 2, 128), U32),
            pltpu.VMEM((2, HIST + SEG, D), F32),
            pltpu.VMEM((2, HIST + SEG, D), F32),
            pltpu.SemaphoreType.DMA((5,)),
            pltpu.SemaphoreType.DMA((NCH, 4)),
            pltpu.SemaphoreType.DMA((1,)),
        ],
        compiler_params=pltpu.CompilerParams(vmem_limit_bytes=120 * 1024 * 1024),
        name="interleaved_rmt_dilated",
    )(A_x.reshape(S, D), A_mem0.reshape(M, D), wt(A_Wq), wt(A_Wk), wt(A_Wv),
      A_Wo.reshape(H * DH, D), B_wqkv, B_wo)
    return out.reshape(1, S, D)
```

```python
import functools

import jax
import jax.numpy as jnp
from jax import lax
import jax.experimental.pallas as pl
import jax.experimental.pallas.tpu as pltpu

F32 = jnp.float32
BF16 = jnp.bfloat16
U32 = jnp.uint32

S = 2048
D = 640
SEG = 32
M = 8
NSEG = S // SEG
L = SEG + M
H = 32
DH = 192
NP = H // 2
PR = 2 * DH
NCH = NP // 2
CR = 2 * PR
KT = D // 128
BW = 8
BDIL = 2
BDH = D // H
HIST = 16
NEG = -1000000000.0
EPS = 1e-5
NSLOT = 3
AHEAD = 2
LAG = 2
BCOUNT = (10, 8, 2, 2, 2, 4, 2, 2, 4, 0, 0, 0, 2, 4, 2, 2, 3)
SCHEDULE = "S3b-1 K0 K1 K2 Q0 K3 S3a-1 B PVa-1 K4 Q1 PVb-1 KPb Q2 Q3 B Q4 B KPa O0-1 V0 QKa O1-1 V1 QKb S1b V2 V3 O2-1 V4 S2b O3-1 S1a O4-1 S2a VPa VPb"


def _bf(x):
    return pltpu.bitcast(x, BF16)


def _u32(x):
    return pltpu.bitcast(x, U32)


def _dot(a, b):
    return lax.dot_general(a, b, (((1,), (0,)), ((), ())), preferred_element_type=F32)


def _dot_t(a, b):
    return lax.dot_general(a, b, (((1,), (1,)), ((), ())), preferred_element_type=F32)


def _layernorm(x):
    m = jnp.sum(x, axis=-1, keepdims=True) * (1.0 / D)
    c = x - m
    v = jnp.sum(c * c, axis=-1, keepdims=True) * (1.0 / D)
    return c * lax.rsqrt(v + EPS)


def _recip(l):
    r = pl.reciprocal(l, approx=True)
    return r * (2.0 - l * r)


_U = (
    ( 0,  0, -1,  0,  0,  0,  0,  1,  0,  0),
    ( 1,  0,  0,  0, -1, -1,  0,  0,  0,  1),
    ( 0,  0,  0,  0,  0,  0, -1,  0,  0,  0),
    ( 0,  0,  0,  1,  0,  0,  0,  0, -1,  0),
    ( 0, -1,  0,  1,  0,  0,  0,  0,  0,  0),
    ( 0,  0, -1,  0,  0,  0,  0,  0,  0,  0),
    ( 0,  0,  0,  1,  1,  0,  0,  0, -1, -1),
    (-1,  0,  0,  0,  1,  1,  0,  0,  0,  0),
    ( 0,  0,  0,  0,  0, -1,  0,  0,  0,  0),
    ( 0,  1,  0,  0,  0,  0, -1,  0,  0,  0),
    ( 0,  0,  0, -1,  0,  0,  1,  0,  0,  0),
    (-1,  0, -1,  0,  0,  0,  0,  0,  0,  0),
    ( 1,  0,  0,  0,  0, -1,  0,  0,  0,  0),
    ( 0,  0,  0,  0,  0,  0,  1,  0, -1,  0),
    ( 0,  0,  0,  0,  0,  1,  0,  1,  0,  0),
    ( 0,  0,  0,  0, -1,  0,  0,  0,  0,  0),
    ( 0,  0,  1,  0,  0,  0, -1,  0,  0,  0),
    ( 0,  0,  0, -1,  0,  0,  0,  0,  1,  1),
    ( 0,  0,  0,  0,  0,  0,  0,  0, -1, -1),
    ( 0,  0,  0,  0,  0,  0,  0,  0,  0, -1),
    ( 0,  0,  0,  0,  0,  0, -1,  1,  0,  0),
    ( 0, -1,  1,  0,  0,  0,  0,  0,  0,  0),
    ( 0,  0, -1,  0,  0, -1,  0,  0,  0,  0),
    ( 0,  0,  0,  1,  0,  0,  0,  0,  0,  0),
    ( 1,  0,  0,  0, -1,  0,  0,  0,  0,  0),
)
_V = (
    ( 0,  0,  0,  0,  0,  0,  1,  0,  1,  0,  0,  0,  0,  0,  0),
    ( 0,  0,  0,  0,  0,  0,  0,  0,  0,  0,  0,  0,  1,  0, -1),
    ( 0,  0,  0,  0,  0, -1,  0,  0, -1,  1,  0, -1,  0,  0,  0),
    ( 0,  0,  0,  0,  0,  0,  0,  0,  0, -1, -1,  1,  0,  1,  0),
    ( 0,  0,  0,  1,  1,  0,  0,  0,  0,  0,  0,  0,  0,  0,  0),
    ( 0,  1,  0,  1,  0,  0,  0, -1,  0,  0,  0,  0,  0,  0,  0),
    ( 0,  0,  0,  0,  0,  0,  0,  0,  0,  0,  0,  0,  0,  1,  0),
    ( 0,  0, -1,  0,  0,  0,  0,  0,  0,  0,  0,  0,  1,  0, -1),
    ( 1,  1,  0,  0,  0,  0, -1, -1,  0,  0,  0,  0,  0,  0,  0),
    ( 0,  0,  0,  0,  1, -1,  0,  0,  0,  0,  0,  0,  0,  0,  0),
    ( 0,  0,  0,  1,  1,  0,  0,  0,  0, -1,  0,  1,  0,  0,  0),
    ( 0, -1,  0,  0,  0,  0,  0,  0,  0,  0,  0,  0,  0,  0,  0),
    ( 1,  0, -1,  0,  0,  0,  0,  0,  0,  0,  0,  0,  1,  0, -1),
    ( 0,  0,  0,  0,  0,  0,  0,  0,  0,  1,  0, -1,  0,  0,  0),
    ( 0,  0,  0,  0,  0,  0,  1,  1,  0,  0,  0,  0,  0,  0,  0),
    ( 0,  0,  1,  0,  0,  0,  0,  0,  0,  0,  0,  0,  0, -1,  1),
    ( 0,  0,  0, -1,  0,  0,  0,  0,  1,  0,  0,  0,  0,  0,  0),
    ( 0,  0,  0,  0,  0,  0,  0,  0,  0, -1,  0,  0,  0,  1,  0),
    ( 0,  0,  0,  0,  0,  0,  0,  0,  0,  1,  0,  0,  0,  0,  0),
    ( 0,  0,  0,  0,  0,  0,  0,  0,  0, -1,  0,  0,  1,  0,  0),
    ( 0,  0,  0,  0,  0,  0,  0,  0,  1,  0,  0,  0,  0,  0,  0),
    ( 0,  0,  0, -1,  0,  0,  0,  0,  0,  0,  0,  0,  0,  0,  0),
    ( 0,  1,  0,  0,  0,  0, -1, -1,  0,  0,  0,  0,  0,  0,  0),
    ( 0,  0,  0, -1, -1,  0,  0,  0,  0,  1, -1,  0,  0,  0,  0),
    ( 0,  0,  1,  0,  0,  0,  0,  0,  0,  0,  0,  0,  0,  0,  0),
)
_W = (
    ( 0,  0,  0,  1, -1,  0),
    ( 0,  0,  0,  0,  0, -1),
    ( 0,  0,  1,  0,  0,  1),
    ( 0,  0,  0,  0,  1,  0),
    ( 0, -1, -1,  0,  0,  0),
    (-1,  1,  0, -1,  1,  0),
    ( 1,  1,  1,  0,  0,  0),
    ( 1,  0,  0,  0,  0, -1),
    (-1,  0,  0, -1,  0,  0),
    ( 0,  0, -1,  0,  0,  0),
    ( 0,  0, -1,  0,  1,  0),
    ( 0,  1,  0,  0,  0,  0),
    ( 1,  0,  0,  0,  0,  0),
    ( 0,  0,  0,  0,  1,  1),
    ( 0,  0,  0,  0,  1,  0),
    (-1,  0, -1,  0,  0,  0),
    ( 0,  0,  1,  1, -1,  0),
    ( 1,  1,  1,  0,  1,  0),
    (-1, -1, -1, -1, -1, -1),
    ( 0,  0,  0, -1,  0, -1),
    ( 0,  0,  0, -1,  1,  1),
    ( 1, -1, -1,  0,  0,  0),
    ( 1,  0,  0,  1, -1,  0),
    ( 0, -1,  0,  0, -1,  0),
    ( 0,  0,  1,  0,  0,  1),
)
NR = len(_U)
NPART = 5


def _comb(coefs, blocks):
    acc = None
    for c, blk in zip(coefs, blocks):
        if c == 0 or blk is None:
            continue
        if acc is None:
            acc = blk if c > 0 else -blk
        else:
            acc = acc + blk if c > 0 else acc - blk
    return acc


def _needed(live):
    return [r for r in range(NR)
            if any(_U[r][5 * m + j] for m in live for j in range(5))
            and any(_W[r][3 * m + k] for m in live for k in range(3))]


def _parts(seq):
    n = len(seq)
    return [seq[(n * i) // NPART:(n * (i + 1)) // NPART] for i in range(NPART)]


def _kernel(x_hbm, mem0_hbm, wqt_hbm, wkt_hbm, wvt_hbm, wo_hbm, bqkv_hbm, bwo_hbm,
            out_ref,
            xs, mem_s, x_s, h_s, stage, ws, wso, lhs, accm,
            bst_qkv, bst_o, bqkv, bwo, kwin, vwin,
            sem_small, sem_a, sem_out):
    def seg_rows(seg):
        if isinstance(seg, int):
            return pl.ds(seg * SEG, SEG)
        return pl.ds(pl.multiple_of(seg * SEG, SEG), SEG)

    def a_copies(c):
        rows = pl.ds(c * CR, CR)
        return [pltpu.make_async_copy(src.at[rows, :], stage.at[c % NSLOT, w], sem_a.at[c, w])
                for w, src in enumerate((wqt_hbm, wkt_hbm, wvt_hbm, wo_hbm))]

    def input_layernorm(seg):
        r = seg_rows(seg)
        h_s[r, :] = _layernorm(xs[r, :].astype(F32))

    ri = lax.broadcasted_iota(jnp.int32, (D, D), 0)
    ci = lax.broadcasted_iota(jnp.int32, (D, D), 1)

    def permute_qkv(part):
        perm = jnp.where(ri == (ci & 31) * BDH + (ci >> 5), 1.0, 0.0).astype(BF16)
        wp = _dot(bst_qkv[:, part * D:(part + 1) * D], perm).astype(BF16)
        for j in range(KT):
            bqkv[part * KT + j] = _u32(wp[:, j * 128:(j + 1) * 128])

    def permute_wo():
        permt = jnp.where(ci == (ri & 31) * BDH + (ri >> 5), 1.0, 0.0).astype(BF16)
        wp = _dot(permt, bst_o[...]).astype(BF16)
        for j in range(KT):
            bwo[j] = _u32(wp[:, j * 128:(j + 1) * 128])

    def build_chunk(c):
        slot = c % NSLOT
        ei = lax.broadcasted_iota(jnp.int32, (128, 128), 0)
        ej = lax.broadcasted_iota(jnp.int32, (128, 128), 1)
        eye = jnp.where(ei == ej, 1.0, 0.0).astype(BF16)

        def qkv_block(n, _):
            w = n // 2
            pp = n % 2
            g = w * NP + 2 * c + pp
            tiles = []
            for j in range(KT):
                for k in range(3):
                    r = pl.ds(pl.multiple_of(pp * PR + k * 128, 128), 128)
                    t = stage[slot, w, r, j * 128:(j + 1) * 128]
                    tiles.append(t.T.astype(F32) if (j * 3 + k) % 2 else _dot_t(eye, t))
            for r in range(NR):
                ws[g, 64 * r:64 * (r + 1), :] = _u32(_comb(_V[r], tiles).astype(BF16))
            return 0
        lax.fori_loop(0, 6, qkv_block, 0)

        def o_block(n, _):
            pp = n // 2
            half = n % 2
            for i in range(4):
                tiles = []
                for j in range(KT):
                    for k in range(3):
                        r = pl.ds(pl.multiple_of(pp * PR + k * 128 + half * 64 + i * 16, 16), 16)
                        tiles.append(stage[slot, 3, r, j * 128:(j + 1) * 128].astype(F32))
                for r in range(NR):
                    wso[2 * c + pp, pl.ds(pl.multiple_of(64 * r + 32 * half + 8 * i, 8), 8), :] = (
                        _u32(_comb(_V[r], tiles).astype(BF16)))
            return 0
        lax.fori_loop(0, 4, o_block, 0)

    XH = 2 * SEG
    items = [
        ([pltpu.make_async_copy(x_hbm.at[pl.ds(0, XH), :], xs.at[pl.ds(0, XH), :], sem_small.at[0]),
          pltpu.make_async_copy(mem0_hbm, mem_s, sem_small.at[1])],
         [functools.partial(input_layernorm, 0)]),
        ([pltpu.make_async_copy(bqkv_hbm, bst_qkv, sem_small.at[2]),
          pltpu.make_async_copy(bwo_hbm, bst_o, sem_small.at[3])], [functools.partial(permute_qkv, 0)]),
    ]
    extra = [functools.partial(permute_qkv, 1), functools.partial(permute_qkv, 2), permute_wo]
    for c in range(NCH):
        work = [functools.partial(build_chunk, c)]
        if c < len(extra):
            work.append(extra[c])
        items.append((a_copies(c), work))
    items.append(([pltpu.make_async_copy(x_hbm.at[pl.ds(XH, S - XH), :], xs.at[pl.ds(XH, S - XH), :],
                                         sem_small.at[4])], []))

    def run_item(n):
        copies, work = items[n]
        if n + AHEAD < len(items):
            for cp in items[n + AHEAD][0]:
                cp.start()
        for cp in copies:
            cp.wait()
        for fn in work:
            fn()

    for copies, _ in items[:AHEAD]:
        for cp in copies:
            cp.start()

    kwin[...] = jnp.zeros(kwin.shape, F32)
    vwin[...] = jnp.zeros(vwin.shape, F32)
    x_s[pl.ds(S, SEG), :] = jnp.zeros((SEG, D), F32)
    xs[pl.ds(S, SEG), :] = jnp.zeros((SEG, D), BF16)
    run_item(0)
    run_item(1)

    mem0 = mem_s[...].astype(F32)

    lane = lax.broadcasted_iota(jnp.int32, (L, 128), 1)
    lo_half = lane < 64
    arow = lax.broadcasted_iota(jnp.int32, (L, 2 * L), 0)
    acol = lax.broadcasted_iota(jnp.int32, (L, 2 * L), 1)
    akey = jnp.where(acol < L, acol, acol - L)
    allowed = (arow >= SEG) | (akey >= SEG) | (akey <= arow)
    mask_e = allowed & (acol < L)
    mask_o = allowed & (acol >= L)
    a_scale = DH ** -0.5
    b_scale = BDH ** -0.5
    brow = lax.broadcasted_iota(jnp.int32, (SEG, 128), 0)

    def b_stages(s1, s2):
        live = [n for n, sg in enumerate((s1, s2)) if sg is not None]
        if not live:
            return
        segs = {n: (s1, s2)[n] for n in live}
        rows = {n: seg_rows(segs[n]) for n in live}
        off_of = {n: i * SEG for i, n in enumerate(live)}
        hn = jnp.concatenate([_layernorm(x_s[rows[n], :]) for n in live], axis=0)
        for n in live:
            kwin[n, 0:HIST, :] = kwin[n, SEG:SEG + HIST, :]
            vwin[n, 0:HIST, :] = vwin[n, SEG:SEG + HIST, :]
        yield
        q = []
        for j in range(KT):
            cols = slice(j * 128, (j + 1) * 128)
            k = _dot(hn, _bf(bqkv[KT + j]))
            for n in live:
                kwin[n, HIST:, cols] = k[off_of[n]:off_of[n] + SEG]
            yield
        for j in range(KT):
            q.append(_dot(hn, _bf(bqkv[j])))
            yield
        for j in range(KT):
            cols = slice(j * 128, (j + 1) * 128)
            v = _dot(hn, _bf(bqkv[2 * KT + j]))
            for n in live:
                vwin[n, HIST:, cols] = v[off_of[n]:off_of[n] + SEG]
            yield
        o = {n: [None] * KT for n in live}
        for n in live:
            pos = brow + segs[n] * SEG
            logits = []
            for w in range(BW):
                off = HIST - BDIL * w
                t = None
                for j in range(KT):
                    cols = slice(j * 128, (j + 1) * 128)
                    pj = q[j][off_of[n]:off_of[n] + SEG] * kwin[n, off:off + SEG, cols]
                    t = pj if t is None else t + pj
                t = t + pltpu.roll(t, 64, axis=1)
                t = t + pltpu.roll(t, 32, axis=1)
                logits.append(jnp.where(pos >= BDIL * w, t * b_scale, NEG))
                yield
            m = logits[0]
            for w in range(1, BW):
                m = jnp.maximum(m, logits[w])
            e = [jnp.exp(lg - m) for lg in logits]
            l = e[0]
            for w in range(1, BW):
                l = l + e[w]
            rl = _recip(l)
            a = [ew * rl for ew in e]
            yield
            for j in range(KT):
                cols = slice(j * 128, (j + 1) * 128)
                t = None
                for w in range(BW):
                    off = HIST - BDIL * w
                    pw = a[w] * vwin[n, off:off + SEG, cols]
                    t = pw if t is None else t + pw
                o[n][j] = t
                yield
        o = jnp.concatenate([jnp.concatenate(o[n], axis=1) for n in live], axis=0)
        y = []
        for j in range(KT):
            y.append(_dot(o, _bf(bwo[j])))
            yield
        y = jnp.concatenate(y, axis=1)
        for n in live:
            xn = x_s[rows[n], :] + y[off_of[n]:off_of[n] + SEG]
            x_s[rows[n], :] = xn
            if n == 0:
                h_s[rows[n], :] = _layernorm(xn)
            else:
                xs[rows[n], :] = xn.astype(BF16)
        yield

    def advance(gen, n):
        for _ in range(n):
            next(gen, None)

    def a_layers(h1, h2, bgen, weights_ready=None):
        live = [m for m, h in enumerate((h1, h2)) if h is not None]
        need = _needed(live)
        parts = _parts(need)
        inst = [dict() for _ in range(2 * NP)]
        hb = [None if h is None else h[:, 128 * j:128 * (j + 1)] for h in (h1, h2) for j in range(KT)]
        for r in need:
            lhs[r] = _comb(_U[r], hb)
        yb = [None] * (2 * KT)

        def pack_kv(t):
            ac = jnp.concatenate([t[0], t[2]], axis=0).astype(BF16)
            bb = jnp.concatenate([jnp.where(lo_half, t[1], 0.0),
                                  jnp.where(lo_half, 0.0, t[1])], axis=0).astype(BF16)
            return ac, bb

        def run(op, p):
            if op[0] in "KQV" and op[1].isdigit():
                g = "QKV".index(op[0]) * NP + p
                c = inst[2 * p].setdefault("c" + op[0], [None] * 6)
                for r in parts[int(op[1])]:
                    mr = _dot(lhs[r], _bf(ws[g, 64 * r:64 * (r + 1), :]))
                    for o in range(6):
                        if o // 3 in live and _W[r][o]:
                            c[o] = _comb((1, _W[r][o]), (c[o], mr))
                if int(op[1]) == NPART - 1:
                    for m in live:
                        inst[2 * p + m][op[0]] = c[3 * m:3 * m + 3]
                    del inst[2 * p]["c" + op[0]]
                return
            if op[0] == "O" and op[1].isdigit():
                d = inst[2 * p]
                if "ob" not in d:
                    d["ob"] = [inst[2 * p + m].pop("o") if m in live else [None] * 3 for m in range(2)]
                    d["ob"] = d["ob"][0] + d["ob"][1]
                for r in parts[int(op[1])]:
                    mr = _dot(_comb(_W[r], d["ob"]), _bf(wso[p, 64 * r:64 * (r + 1), :]))
                    if p == 0:
                        accm[r] = mr
                    elif p < NP - 1:
                        accm[r] = accm[r] + mr
                    else:
                        mr = accm[r] + mr
                        for a in range(2 * KT):
                            if a // KT in live and _U[r][a]:
                                yb[a] = _comb((1, _U[r][a]), (yb[a], mr))
                return
            if "ab".index(op[2]) not in live:
                return
            d = inst[2 * p + "ab".index(op[2])]
            op = op[:2]
            if op == "KP":
                d["kp"] = pack_kv(d.pop("K"))
            elif op == "VP":
                d["vp"] = pack_kv(d.pop("V"))
            elif op == "QK":
                q = d.pop("Q")
                k_ac, k_b = d.pop("kp")
                d["sc"] = (_dot_t(jnp.concatenate([q[0], q[2]], axis=0), k_ac), _dot_t(q[1], k_b))
            elif op == "S1":
                s_ac, s_b = d.pop("sc")
                s_e = jnp.where(mask_e, (s_ac[:L] + s_b) * a_scale, NEG)
                s_o = jnp.where(mask_o, (s_ac[L:] + s_b) * a_scale, NEG)
                d["mx"] = [(s, jnp.max(s, axis=-1, keepdims=True)) for s in (s_e, s_o)]
            elif op == "S2":
                es = [jnp.exp(s - m) for s, m in d.pop("mx")]
                d["pr"] = [(e, jnp.sum(e, axis=-1, keepdims=True)) for e in es]
            elif op == "S3":
                d["p"] = [e * _recip(l) for e, l in d.pop("pr")]
            elif op == "PV":
                p_e, p_o = d.pop("p")
                v_ac, v_b = d.pop("vp")
                o_ac = _dot(jnp.concatenate([p_e, p_o], axis=0), v_ac)
                o_b = _dot(p_e + p_o, v_b)
                d["o"] = [o_ac[:L], o_b, o_ac[L:]]
            else:
                raise ValueError(op)

        toks = SCHEDULE.split()
        maxlag = max(int(t.partition("-")[2] or 0) for t in toks)
        nb = toks.count("B")
        for i in range(NP + maxlag):
            if weights_ready is not None and i < NP and i % 2 == 0:
                weights_ready(i // 2)
            bi = 0
            for tok in toks:
                if tok == "B":
                    n = BCOUNT[i] if i < len(BCOUNT) else 0
                    advance(bgen, (n * (bi + 1)) // nb - (n * bi) // nb)
                    bi += 1
                    continue
                op, _, lag = tok.partition("-")
                p = i - int(lag or 0)
                if 0 <= p < NP:
                    run(op, p)
        return [jnp.concatenate(yb[KT * m:KT * (m + 1)], axis=1) if m in live else None for m in range(2)]

    def out_copy(seg):
        r = seg_rows(seg)
        return pltpu.make_async_copy(xs.at[r, :], out_ref.at[r, :], sem_out.at[0])

    def step(t, carry, first=False):
        mem1, mem2 = carry
        static = isinstance(t, int)
        valid = lambda sg: sg if (not static or 0 <= sg < NSEG) else None
        s1, s2, sb1, sb2 = valid(t), valid(t - LAG), valid(t - 1), valid(t - LAG - 1)
        if not static:
            sb2 = jnp.where(sb2 < 0, NSEG, sb2)
        h1 = None if s1 is None else jnp.concatenate([h_s[seg_rows(s1), :], mem1], axis=0)
        h2 = None if s2 is None else jnp.concatenate([h_s[seg_rows(s2), :], mem2], axis=0)
        bgen = b_stages(sb1, sb2)
        if s1 is not None and (not static or s1 + 1 < NSEG):
            input_layernorm(s1 + 1)
        y1, y2 = a_layers(h1, h2, bgen, (lambda c: run_item(2 + c)) if first else None)
        advance(bgen, 1000)
        if s1 is not None:
            x_s[seg_rows(s1), :] = xs[seg_rows(s1), :].astype(F32) + y1[:SEG]
            mem1 = y1[SEG:]
        if s2 is not None:
            x_s[seg_rows(s2), :] = x_s[seg_rows(s2), :] + y2[:SEG]
            mem2 = y2[SEG:]
        if static:
            if sb2 is not None:
                out_copy(sb2).start()
        else:
            @pl.when(t - LAG - 1 >= 0)
            def _():
                out_copy(t - LAG - 1).start()
        return mem1, mem2

    carry = step(0, (mem0, mem0), first=True)
    run_item(len(items) - 1)
    for t in range(1, LAG):
        carry = step(t, carry)
    carry = lax.fori_loop(LAG, NSEG, step, carry)
    for t in range(NSEG, NSEG + LAG):
        carry = step(t, carry)
    advance(b_stages(None, NSEG - 1), 1000)
    out_copy(NSEG - 1).start()

    def wait_out(i, _):
        out_copy(i).wait()
        return 0
    lax.fori_loop(0, NSEG, wait_out, 0)


@functools.partial(jax.jit, static_argnames=("A_seg_len",))
def pallas_interleave_layers__memory_aug_recurrent_mem_tr__sliding_local_dilated__prompt_kernel(
    A_x, A_mem0, A_Wq, A_Wk, A_Wv, A_Wo, A_seg_len, B_x, B_wqkv, B_wo,
):
    del B_x
    assert int(A_seg_len) == SEG
    assert A_x.shape == (1, S, D) and A_mem0.shape == (1, M, D)
    assert A_Wq.shape == (D, H, DH) and A_Wo.shape == (H, DH, D)

    def wt(w):
        return jnp.transpose(w, (1, 2, 0)).reshape(H * DH, D)

    any_spec = pl.BlockSpec(memory_space=pl.ANY)
    out = pl.pallas_call(
        _kernel,
        out_shape=jax.ShapeDtypeStruct((S, D), BF16),
        in_specs=[any_spec] * 8,
        out_specs=any_spec,
        scratch_shapes=[
            pltpu.VMEM((S + SEG, D), BF16),
            pltpu.VMEM((M, D), BF16),
            pltpu.VMEM((S + SEG, D), F32),
            pltpu.VMEM((S + SEG, D), F32),
            pltpu.VMEM((NSLOT, 4, CR, D), BF16),
            pltpu.VMEM((3 * NP, NR * 64, 128), U32),
            pltpu.VMEM((NP, NR * 64, 128), U32),
            pltpu.VMEM((NR, L, 128), F32),
            pltpu.VMEM((NR, L, 128), F32),
            pltpu.VMEM((D, 3 * D), BF16),
            pltpu.VMEM((D, D), BF16),
            pltpu.VMEM((3 * KT, D // 2, 128), U32),
            pltpu.VMEM((KT, D // 2, 128), U32),
            pltpu.VMEM((2, HIST + SEG, D), F32),
            pltpu.VMEM((2, HIST + SEG, D), F32),
            pltpu.SemaphoreType.DMA((5,)),
            pltpu.SemaphoreType.DMA((NCH, 4)),
            pltpu.SemaphoreType.DMA((1,)),
        ],
        compiler_params=pltpu.CompilerParams(vmem_limit_bytes=120 * 1024 * 1024),
        name="interleaved_rmt_dilated",
    )(A_x.reshape(S, D), A_mem0.reshape(M, D), wt(A_Wq), wt(A_Wk), wt(A_Wv),
      A_Wo.reshape(H * DH, D), B_wqkv, B_wo)
    return out.reshape(1, S, D)
```

```python
import functools

import jax
import jax.numpy as jnp
from jax import lax
import jax.experimental.pallas as pl
import jax.experimental.pallas.tpu as pltpu

F32 = jnp.float32
BF16 = jnp.bfloat16
U32 = jnp.uint32

S = 2048
D = 640
SEG = 32
M = 8
NSEG = S // SEG
L = SEG + M
H = 32
DH = 192
NP = H // 2
PR = 2 * DH
NCH = NP // 2
CR = 2 * PR
KT = D // 128
BW = 8
BDIL = 2
BDH = D // H
HIST = 16
NEG = -1000000000.0
EPS = 1e-5
NSLOT = 3
AHEAD = 2
LAG = 2
BCOUNT = (10, 8, 2, 2, 3, 4, 2, 2, 4, 0, 0, 0, 2, 4, 1, 2, 3)
SCHEDULE = "S3b-1 K0 K1 K2 Q0 K3 S3a-1 B PVa-1 K4 Q1 PVb-1 KPb Q2 Q3 B Q4 KPa B O0-1 V0 QKa O1-1 V1 QKb S1b V2 V3 V4 O2-1 S2b O3-1 S1a VPb O4-1 VPa S2a"


def _bf(x):
    return pltpu.bitcast(x, BF16)


def _u32(x):
    return pltpu.bitcast(x, U32)


def _dot(a, b):
    return lax.dot_general(a, b, (((1,), (0,)), ((), ())), preferred_element_type=F32)


def _dot_t(a, b):
    return lax.dot_general(a, b, (((1,), (1,)), ((), ())), preferred_element_type=F32)


def _layernorm(x):
    m = jnp.sum(x, axis=-1, keepdims=True) * (1.0 / D)
    c = x - m
    v = jnp.sum(c * c, axis=-1, keepdims=True) * (1.0 / D)
    return c * lax.rsqrt(v + EPS)


def _recip(l):
    r = pl.reciprocal(l, approx=True)
    return r * (2.0 - l * r)


_U = (
    ( 0,  0, -1,  0,  0,  0,  0,  1,  0,  0),
    ( 1,  0,  0,  0, -1, -1,  0,  0,  0,  1),
    ( 0,  0,  0,  0,  0,  0, -1,  0,  0,  0),
    ( 0,  0,  0,  1,  0,  0,  0,  0, -1,  0),
    ( 0, -1,  0,  1,  0,  0,  0,  0,  0,  0),
    ( 0,  0, -1,  0,  0,  0,  0,  0,  0,  0),
    ( 0,  0,  0,  1,  1,  0,  0,  0, -1, -1),
    (-1,  0,  0,  0,  1,  1,  0,  0,  0,  0),
    ( 0,  0,  0,  0,  0, -1,  0,  0,  0,  0),
    ( 0,  1,  0,  0,  0,  0, -1,  0,  0,  0),
    ( 0,  0,  0, -1,  0,  0,  1,  0,  0,  0),
    (-1,  0, -1,  0,  0,  0,  0,  0,  0,  0),
    ( 1,  0,  0,  0,  0, -1,  0,  0,  0,  0),
    ( 0,  0,  0,  0,  0,  0,  1,  0, -1,  0),
    ( 0,  0,  0,  0,  0,  1,  0,  1,  0,  0),
    ( 0,  0,  0,  0, -1,  0,  0,  0,  0,  0),
    ( 0,  0,  1,  0,  0,  0, -1,  0,  0,  0),
    ( 0,  0,  0, -1,  0,  0,  0,  0,  1,  1),
    ( 0,  0,  0,  0,  0,  0,  0,  0, -1, -1),
    ( 0,  0,  0,  0,  0,  0,  0,  0,  0, -1),
    ( 0,  0,  0,  0,  0,  0, -1,  1,  0,  0),
    ( 0, -1,  1,  0,  0,  0,  0,  0,  0,  0),
    ( 0,  0, -1,  0,  0, -1,  0,  0,  0,  0),
    ( 0,  0,  0,  1,  0,  0,  0,  0,  0,  0),
    ( 1,  0,  0,  0, -1,  0,  0,  0,  0,  0),
)
_V = (
    ( 0,  0,  0,  0,  0,  0,  1,  0,  1,  0,  0,  0,  0,  0,  0),
    ( 0,  0,  0,  0,  0,  0,  0,  0,  0,  0,  0,  0,  1,  0, -1),
    ( 0,  0,  0,  0,  0, -1,  0,  0, -1,  1,  0, -1,  0,  0,  0),
    ( 0,  0,  0,  0,  0,  0,  0,  0,  0, -1, -1,  1,  0,  1,  0),
    ( 0,  0,  0,  1,  1,  0,  0,  0,  0,  0,  0,  0,  0,  0,  0),
    ( 0,  1,  0,  1,  0,  0,  0, -1,  0,  0,  0,  0,  0,  0,  0),
    ( 0,  0,  0,  0,  0,  0,  0,  0,  0,  0,  0,  0,  0,  1,  0),
    ( 0,  0, -1,  0,  0,  0,  0,  0,  0,  0,  0,  0,  1,  0, -1),
    ( 1,  1,  0,  0,  0,  0, -1, -1,  0,  0,  0,  0,  0,  0,  0),
    ( 0,  0,  0,  0,  1, -1,  0,  0,  0,  0,  0,  0,  0,  0,  0),
    ( 0,  0,  0,  1,  1,  0,  0,  0,  0, -1,  0,  1,  0,  0,  0),
    ( 0, -1,  0,  0,  0,  0,  0,  0,  0,  0,  0,  0,  0,  0,  0),
    ( 1,  0, -1,  0,  0,  0,  0,  0,  0,  0,  0,  0,  1,  0, -1),
    ( 0,  0,  0,  0,  0,  0,  0,  0,  0,  1,  0, -1,  0,  0,  0),
    ( 0,  0,  0,  0,  0,  0,  1,  1,  0,  0,  0,  0,  0,  0,  0),
    ( 0,  0,  1,  0,  0,  0,  0,  0,  0,  0,  0,  0,  0, -1,  1),
    ( 0,  0,  0, -1,  0,  0,  0,  0,  1,  0,  0,  0,  0,  0,  0),
    ( 0,  0,  0,  0,  0,  0,  0,  0,  0, -1,  0,  0,  0,  1,  0),
    ( 0,  0,  0,  0,  0,  0,  0,  0,  0,  1,  0,  0,  0,  0,  0),
    ( 0,  0,  0,  0,  0,  0,  0,  0,  0, -1,  0,  0,  1,  0,  0),
    ( 0,  0,  0,  0,  0,  0,  0,  0,  1,  0,  0,  0,  0,  0,  0),
    ( 0,  0,  0, -1,  0,  0,  0,  0,  0,  0,  0,  0,  0,  0,  0),
    ( 0,  1,  0,  0,  0,  0, -1, -1,  0,  0,  0,  0,  0,  0,  0),
    ( 0,  0,  0, -1, -1,  0,  0,  0,  0,  1, -1,  0,  0,  0,  0),
    ( 0,  0,  1,  0,  0,  0,  0,  0,  0,  0,  0,  0,  0,  0,  0),
)
_W = (
    ( 0,  0,  0,  1, -1,  0),
    ( 0,  0,  0,  0,  0, -1),
    ( 0,  0,  1,  0,  0,  1),
    ( 0,  0,  0,  0,  1,  0),
    ( 0, -1, -1,  0,  0,  0),
    (-1,  1,  0, -1,  1,  0),
    ( 1,  1,  1,  0,  0,  0),
    ( 1,  0,  0,  0,  0, -1),
    (-1,  0,  0, -1,  0,  0),
    ( 0,  0, -1,  0,  0,  0),
    ( 0,  0, -1,  0,  1,  0),
    ( 0,  1,  0,  0,  0,  0),
    ( 1,  0,  0,  0,  0,  0),
    ( 0,  0,  0,  0,  1,  1),
    ( 0,  0,  0,  0,  1,  0),
    (-1,  0, -1,  0,  0,  0),
    ( 0,  0,  1,  1, -1,  0),
    ( 1,  1,  1,  0,  1,  0),
    (-1, -1, -1, -1, -1, -1),
    ( 0,  0,  0, -1,  0, -1),
    ( 0,  0,  0, -1,  1,  1),
    ( 1, -1, -1,  0,  0,  0),
    ( 1,  0,  0,  1, -1,  0),
    ( 0, -1,  0,  0, -1,  0),
    ( 0,  0,  1,  0,  0,  1),
)
NR = len(_U)
ORDER_P = (0, 1, 2, 3, 4, 5, 21, 6, 11, 7, 8, 9, 10, 13, 14, 15, 16, 17, 12, 18, 19, 20, 22, 23, 24)
ORDER_O = (1, 2, 3, 4, 5, 6, 7, 8, 0, 9, 10, 11, 12, 13, 17, 14, 15, 16, 18, 19, 20, 21, 22, 23, 24)
NPART = 5


def _comb(coefs, blocks):
    acc = None
    for c, blk in zip(coefs, blocks):
        if c == 0 or blk is None:
            continue
        if acc is None:
            acc = blk if c > 0 else -blk
        else:
            acc = acc + blk if c > 0 else acc - blk
    return acc


def _needed(live):
    return [r for r in range(NR)
            if any(_U[r][5 * m + j] for m in live for j in range(5))
            and any(_W[r][3 * m + k] for m in live for k in range(3))]


def _parts(seq):
    n = len(seq)
    return [seq[(n * i) // NPART:(n * (i + 1)) // NPART] for i in range(NPART)]


def _kernel(x_hbm, mem0_hbm, wqt_hbm, wkt_hbm, wvt_hbm, wo_hbm, bqkv_hbm, bwo_hbm,
            out_ref,
            xs, mem_s, x_s, h_s, stage, ws, wso, lhs, accm,
            bst_qkv, bst_o, bqkv, bwo, kwin, vwin,
            sem_small, sem_a, sem_out):
    def seg_rows(seg):
        if isinstance(seg, int):
            return pl.ds(seg * SEG, SEG)
        return pl.ds(pl.multiple_of(seg * SEG, SEG), SEG)

    def a_copies(c):
        rows = pl.ds(c * CR, CR)
        return [pltpu.make_async_copy(src.at[rows, :], stage.at[c % NSLOT, w], sem_a.at[c, w])
                for w, src in enumerate((wqt_hbm, wkt_hbm, wvt_hbm, wo_hbm))]

    def input_layernorm(seg):
        r = seg_rows(seg)
        h_s[r, :] = _layernorm(xs[r, :].astype(F32))

    ri = lax.broadcasted_iota(jnp.int32, (D, D), 0)
    ci = lax.broadcasted_iota(jnp.int32, (D, D), 1)

    def permute_qkv(part):
        perm = jnp.where(ri == (ci & 31) * BDH + (ci >> 5), 1.0, 0.0).astype(BF16)
        wp = _dot(bst_qkv[:, part * D:(part + 1) * D], perm).astype(BF16)
        for j in range(KT):
            bqkv[part * KT + j] = _u32(wp[:, j * 128:(j + 1) * 128])

    def permute_wo():
        permt = jnp.where(ci == (ri & 31) * BDH + (ri >> 5), 1.0, 0.0).astype(BF16)
        wp = _dot(permt, bst_o[...]).astype(BF16)
        for j in range(KT):
            bwo[j] = _u32(wp[:, j * 128:(j + 1) * 128])

    def build_chunk(c):
        slot = c % NSLOT
        ei = lax.broadcasted_iota(jnp.int32, (128, 128), 0)
        ej = lax.broadcasted_iota(jnp.int32, (128, 128), 1)
        eye = jnp.where(ei == ej, 1.0, 0.0).astype(BF16)

        def qkv_block(n, _):
            w = n // 2
            pp = n % 2
            g = w * NP + 2 * c + pp
            tiles = []
            for j in range(KT):
                for k in range(3):
                    r = pl.ds(pl.multiple_of(pp * PR + k * 128, 128), 128)
                    t = stage[slot, w, r, j * 128:(j + 1) * 128]
                    tiles.append(t.T.astype(F32) if (j * 3 + k) % 2 else _dot_t(eye, t))
            for r in range(NR):
                ws[g, 64 * r:64 * (r + 1), :] = _u32(_comb(_V[r], tiles).astype(BF16))
            return 0
        lax.fori_loop(0, 6, qkv_block, 0)

        def o_block(n, _):
            pp = n // 2
            half = n % 2
            for i in range(4):
                tiles = []
                for j in range(KT):
                    for k in range(3):
                        r = pl.ds(pl.multiple_of(pp * PR + k * 128 + half * 64 + i * 16, 16), 16)
                        tiles.append(stage[slot, 3, r, j * 128:(j + 1) * 128].astype(F32))
                for r in range(NR):
                    wso[2 * c + pp, pl.ds(pl.multiple_of(64 * r + 32 * half + 8 * i, 8), 8), :] = (
                        _u32(_comb(_V[r], tiles).astype(BF16)))
            return 0
        lax.fori_loop(0, 4, o_block, 0)

    XH = 2 * SEG
    items = [
        ([pltpu.make_async_copy(x_hbm.at[pl.ds(0, XH), :], xs.at[pl.ds(0, XH), :], sem_small.at[0]),
          pltpu.make_async_copy(mem0_hbm, mem_s, sem_small.at[1])],
         [functools.partial(input_layernorm, 0)]),
        ([pltpu.make_async_copy(bqkv_hbm, bst_qkv, sem_small.at[2]),
          pltpu.make_async_copy(bwo_hbm, bst_o, sem_small.at[3])], [functools.partial(permute_qkv, 0)]),
    ]
    extra = [functools.partial(permute_qkv, 1), functools.partial(permute_qkv, 2), permute_wo]
    for c in range(NCH):
        work = [functools.partial(build_chunk, c)]
        if c < len(extra):
            work.append(extra[c])
        items.append((a_copies(c), work))
    items.append(([pltpu.make_async_copy(x_hbm.at[pl.ds(XH, S - XH), :], xs.at[pl.ds(XH, S - XH), :],
                                         sem_small.at[4])], []))

    def run_item(n):
        copies, work = items[n]
        if n + AHEAD < len(items):
            for cp in items[n + AHEAD][0]:
                cp.start()
        for cp in copies:
            cp.wait()
        for fn in work:
            fn()

    for copies, _ in items[:AHEAD]:
        for cp in copies:
            cp.start()

    kwin[...] = jnp.zeros(kwin.shape, F32)
    vwin[...] = jnp.zeros(vwin.shape, F32)
    x_s[pl.ds(S, SEG), :] = jnp.zeros((SEG, D), F32)
    xs[pl.ds(S, SEG), :] = jnp.zeros((SEG, D), BF16)
    run_item(0)
    run_item(1)

    mem0 = mem_s[...].astype(F32)

    lane = lax.broadcasted_iota(jnp.int32, (L, 128), 1)
    lo_half = lane < 64
    arow = lax.broadcasted_iota(jnp.int32, (L, 2 * L), 0)
    acol = lax.broadcasted_iota(jnp.int32, (L, 2 * L), 1)
    akey = jnp.where(acol < L, acol, acol - L)
    allowed = (arow >= SEG) | (akey >= SEG) | (akey <= arow)
    mask_e = allowed & (acol < L)
    mask_o = allowed & (acol >= L)
    a_scale = DH ** -0.5
    b_scale = BDH ** -0.5
    brow = lax.broadcasted_iota(jnp.int32, (SEG, 128), 0)

    def b_stages(s1, s2):
        live = [n for n, sg in enumerate((s1, s2)) if sg is not None]
        if not live:
            return
        segs = {n: (s1, s2)[n] for n in live}
        rows = {n: seg_rows(segs[n]) for n in live}
        off_of = {n: i * SEG for i, n in enumerate(live)}
        hn = jnp.concatenate([_layernorm(x_s[rows[n], :]) for n in live], axis=0)
        for n in live:
            kwin[n, 0:HIST, :] = kwin[n, SEG:SEG + HIST, :]
            vwin[n, 0:HIST, :] = vwin[n, SEG:SEG + HIST, :]
        yield
        q = []
        for j in range(KT):
            cols = slice(j * 128, (j + 1) * 128)
            k = _dot(hn, _bf(bqkv[KT + j]))
            for n in live:
                kwin[n, HIST:, cols] = k[off_of[n]:off_of[n] + SEG]
            yield
        for j in range(KT):
            q.append(_dot(hn, _bf(bqkv[j])))
            yield
        for j in range(KT):
            cols = slice(j * 128, (j + 1) * 128)
            v = _dot(hn, _bf(bqkv[2 * KT + j]))
            for n in live:
                vwin[n, HIST:, cols] = v[off_of[n]:off_of[n] + SEG]
            yield
        o = {n: [None] * KT for n in live}
        for n in live:
            pos = brow + segs[n] * SEG
            logits = []
            for w in range(BW):
                off = HIST - BDIL * w
                t = None
                for j in range(KT):
                    cols = slice(j * 128, (j + 1) * 128)
                    pj = q[j][off_of[n]:off_of[n] + SEG] * kwin[n, off:off + SEG, cols]
                    t = pj if t is None else t + pj
                t = t + pltpu.roll(t, 64, axis=1)
                t = t + pltpu.roll(t, 32, axis=1)
                logits.append(jnp.where(pos >= BDIL * w, t * b_scale, NEG))
                yield
            m = logits[0]
            for w in range(1, BW):
                m = jnp.maximum(m, logits[w])
            e = [jnp.exp(lg - m) for lg in logits]
            l = e[0]
            for w in range(1, BW):
                l = l + e[w]
            rl = _recip(l)
            a = [ew * rl for ew in e]
            yield
            for j in range(KT):
                cols = slice(j * 128, (j + 1) * 128)
                t = None
                for w in range(BW):
                    off = HIST - BDIL * w
                    pw = a[w] * vwin[n, off:off + SEG, cols]
                    t = pw if t is None else t + pw
                o[n][j] = t
                yield
        o = jnp.concatenate([jnp.concatenate(o[n], axis=1) for n in live], axis=0)
        y = []
        for j in range(KT):
            y.append(_dot(o, _bf(bwo[j])))
            yield
        y = jnp.concatenate(y, axis=1)
        for n in live:
            xn = x_s[rows[n], :] + y[off_of[n]:off_of[n] + SEG]
            x_s[rows[n], :] = xn
            if n == 0:
                h_s[rows[n], :] = _layernorm(xn)
            else:
                xs[rows[n], :] = xn.astype(BF16)
        yield

    def advance(gen, n):
        for _ in range(n):
            next(gen, None)

    def a_layers(h1, h2, bgen, weights_ready=None):
        live = [m for m, h in enumerate((h1, h2)) if h is not None]
        need = _needed(live)
        parts = _parts([r for r in ORDER_P if r in need])
        parts_o = _parts([r for r in ORDER_O if r in need])
        inst = [dict() for _ in range(2 * NP)]
        hb = [None if h is None else h[:, 128 * j:128 * (j + 1)] for h in (h1, h2) for j in range(KT)]
        for r in need:
            lhs[r] = _comb(_U[r], hb)
        yb = [None] * (2 * KT)

        def pack_kv(t):
            ac = jnp.concatenate([t[0], t[2]], axis=0).astype(BF16)
            bb = jnp.concatenate([jnp.where(lo_half, t[1], 0.0),
                                  jnp.where(lo_half, 0.0, t[1])], axis=0).astype(BF16)
            return ac, bb

        def run(op, p):
            if op[0] in "KQV" and op[1].isdigit():
                g = "QKV".index(op[0]) * NP + p
                c = inst[2 * p].setdefault("c" + op[0], [None] * 6)
                for r in parts[int(op[1])]:
                    mr = _dot(lhs[r], _bf(ws[g, 64 * r:64 * (r + 1), :]))
                    for o in range(6):
                        if o // 3 in live and _W[r][o]:
                            c[o] = _comb((1, _W[r][o]), (c[o], mr))
                if int(op[1]) == NPART - 1:
                    for m in live:
                        inst[2 * p + m][op[0]] = c[3 * m:3 * m + 3]
                    del inst[2 * p]["c" + op[0]]
                return
            if op[0] == "O" and op[1].isdigit():
                d = inst[2 * p]
                if "ob" not in d:
                    d["ob"] = [inst[2 * p + m].pop("o") if m in live else [None] * 3 for m in range(2)]
                    d["ob"] = d["ob"][0] + d["ob"][1]
                for r in parts_o[int(op[1])]:
                    mr = _dot(_comb(_W[r], d["ob"]), _bf(wso[p, 64 * r:64 * (r + 1), :]))
                    if p == 0:
                        accm[r] = mr
                    elif p < NP - 1:
                        accm[r] = accm[r] + mr
                    else:
                        mr = accm[r] + mr
                        for a in range(2 * KT):
                            if a // KT in live and _U[r][a]:
                                yb[a] = _comb((1, _U[r][a]), (yb[a], mr))
                return
            if "ab".index(op[2]) not in live:
                return
            d = inst[2 * p + "ab".index(op[2])]
            op = op[:2]
            if op == "KP":
                d["kp"] = pack_kv(d.pop("K"))
            elif op == "VP":
                d["vp"] = pack_kv(d.pop("V"))
            elif op == "QK":
                q = d.pop("Q")
                k_ac, k_b = d.pop("kp")
                d["sc"] = (_dot_t(jnp.concatenate([q[0], q[2]], axis=0), k_ac), _dot_t(q[1], k_b))
            elif op == "S1":
                s_ac, s_b = d.pop("sc")
                s_e = jnp.where(mask_e, (s_ac[:L] + s_b) * a_scale, NEG)
                s_o = jnp.where(mask_o, (s_ac[L:] + s_b) * a_scale, NEG)
                d["mx"] = [(s, jnp.max(s, axis=-1, keepdims=True)) for s in (s_e, s_o)]
            elif op == "S2":
                es = [jnp.exp(s - m) for s, m in d.pop("mx")]
                d["pr"] = [(e, jnp.sum(e, axis=-1, keepdims=True)) for e in es]
            elif op == "S3":
                d["p"] = [e * _recip(l) for e, l in d.pop("pr")]
            elif op == "PV":
                p_e, p_o = d.pop("p")
                v_ac, v_b = d.pop("vp")
                o_ac = _dot(jnp.concatenate([p_e, p_o], axis=0), v_ac)
                o_b = _dot(p_e + p_o, v_b)
                d["o"] = [o_ac[:L], o_b, o_ac[L:]]
            else:
                raise ValueError(op)

        toks = SCHEDULE.split()
        maxlag = max(int(t.partition("-")[2] or 0) for t in toks)
        nb = toks.count("B")
        for i in range(NP + maxlag):
            if weights_ready is not None and i < NP and i % 2 == 0:
                weights_ready(i // 2)
            bi = 0
            for tok in toks:
                if tok == "B":
                    n = BCOUNT[i] if i < len(BCOUNT) else 0
                    advance(bgen, (n * (bi + 1)) // nb - (n * bi) // nb)
                    bi += 1
                    continue
                op, _, lag = tok.partition("-")
                p = i - int(lag or 0)
                if 0 <= p < NP:
                    run(op, p)
        return [jnp.concatenate(yb[KT * m:KT * (m + 1)], axis=1) if m in live else None for m in range(2)]

    def out_copy(seg):
        r = seg_rows(seg)
        return pltpu.make_async_copy(xs.at[r, :], out_ref.at[r, :], sem_out.at[0])

    def step(t, carry, first=False):
        mem1, mem2 = carry
        static = isinstance(t, int)
        valid = lambda sg: sg if (not static or 0 <= sg < NSEG) else None
        s1, s2, sb1, sb2 = valid(t), valid(t - LAG), valid(t - 1), valid(t - LAG - 1)
        if not static:
            sb2 = jnp.where(sb2 < 0, NSEG, sb2)
        h1 = None if s1 is None else jnp.concatenate([h_s[seg_rows(s1), :], mem1], axis=0)
        h2 = None if s2 is None else jnp.concatenate([h_s[seg_rows(s2), :], mem2], axis=0)
        bgen = b_stages(sb1, sb2)
        if s1 is not None and (not static or s1 + 1 < NSEG):
            input_layernorm(s1 + 1)
        y1, y2 = a_layers(h1, h2, bgen, (lambda c: run_item(2 + c)) if first else None)
        advance(bgen, 1000)
        if s1 is not None:
            x_s[seg_rows(s1), :] = xs[seg_rows(s1), :].astype(F32) + y1[:SEG]
            mem1 = y1[SEG:]
        if s2 is not None:
            x_s[seg_rows(s2), :] = x_s[seg_rows(s2), :] + y2[:SEG]
            mem2 = y2[SEG:]
        if static:
            if sb2 is not None:
                out_copy(sb2).start()
        else:
            @pl.when(t - LAG - 1 >= 0)
            def _():
                out_copy(t - LAG - 1).start()
        return mem1, mem2

    carry = step(0, (mem0, mem0), first=True)
    run_item(len(items) - 1)
    for t in range(1, LAG):
        carry = step(t, carry)
    carry = lax.fori_loop(LAG, NSEG, step, carry)
    for t in range(NSEG, NSEG + LAG):
        carry = step(t, carry)
    advance(b_stages(None, NSEG - 1), 1000)
    out_copy(NSEG - 1).start()

    def wait_out(i, _):
        out_copy(i).wait()
        return 0
    lax.fori_loop(0, NSEG, wait_out, 0)


@functools.partial(jax.jit, static_argnames=("A_seg_len",))
def pallas_interleave_layers__memory_aug_recurrent_mem_tr__sliding_local_dilated__prompt_kernel(
    A_x, A_mem0, A_Wq, A_Wk, A_Wv, A_Wo, A_seg_len, B_x, B_wqkv, B_wo,
):
    del B_x
    assert int(A_seg_len) == SEG
    assert A_x.shape == (1, S, D) and A_mem0.shape == (1, M, D)
    assert A_Wq.shape == (D, H, DH) and A_Wo.shape == (H, DH, D)

    def wt(w):
        return jnp.transpose(w, (1, 2, 0)).reshape(H * DH, D)

    any_spec = pl.BlockSpec(memory_space=pl.ANY)
    out = pl.pallas_call(
        _kernel,
        out_shape=jax.ShapeDtypeStruct((S, D), BF16),
        in_specs=[any_spec] * 8,
        out_specs=any_spec,
        scratch_shapes=[
            pltpu.VMEM((S + SEG, D), BF16),
            pltpu.VMEM((M, D), BF16),
            pltpu.VMEM((S + SEG, D), F32),
            pltpu.VMEM((S + SEG, D), F32),
            pltpu.VMEM((NSLOT, 4, CR, D), BF16),
            pltpu.VMEM((3 * NP, NR * 64, 128), U32),
            pltpu.VMEM((NP, NR * 64, 128), U32),
            pltpu.VMEM((NR, L, 128), F32),
            pltpu.VMEM((NR, L, 128), F32),
            pltpu.VMEM((D, 3 * D), BF16),
            pltpu.VMEM((D, D), BF16),
            pltpu.VMEM((3 * KT, D // 2, 128), U32),
            pltpu.VMEM((KT, D // 2, 128), U32),
            pltpu.VMEM((2, HIST + SEG, D), F32),
            pltpu.VMEM((2, HIST + SEG, D), F32),
            pltpu.SemaphoreType.DMA((5,)),
            pltpu.SemaphoreType.DMA((NCH, 4)),
            pltpu.SemaphoreType.DMA((1,)),
        ],
        compiler_params=pltpu.CompilerParams(vmem_limit_bytes=120 * 1024 * 1024),
        name="interleaved_rmt_dilated",
    )(A_x.reshape(S, D), A_mem0.reshape(M, D), wt(A_Wq), wt(A_Wk), wt(A_Wv),
      A_Wo.reshape(H * DH, D), B_wqkv, B_wo)
    return out.reshape(1, S, D)
```
